```python
import jax
import jax.numpy as jnp

def _softmax(x, axis=-1):
    return jax.nn.softmax(x, axis=axis)

def _gelu(x):
    return jax.nn.gelu(x, approximate=True)

def _silu(x):
    return jax.nn.silu(x)

def _sigmoid(x):
    return jax.nn.sigmoid(x)

def _layernorm(x, axis=-1, eps=1e-05):
    m = jnp.mean(x, axis=axis, keepdims=True)
    v = jnp.var(x, axis=axis, keepdims=True)
    return (x - m) / jnp.sqrt(v + eps)

def _scatter_add(tgt, idx, src, axis=0):
    return tgt.at[idx].add(src)

def _segment_sum(src, seg, n):
    return jax.ops.segment_sum(src, seg, n)

class _Rng:

    def __init__(self, key):
        self._k = key

    def _next(self):
        self._k, sub = jax.random.split(self._k)
        return sub

    def normal(self, shape):
        return jax.random.normal(self._next(), shape, dtype=jnp.bfloat16)

    def randint(self, lo, hi, shape):
        return jax.random.randint(self._next(), shape, lo, hi, dtype=jnp.int32)

    def uniform(self, shape, lo=0.0, hi=1.0):
        return jax.random.uniform(self._next(), shape, jnp.bfloat16, lo, hi)

    def permutation(self, n):
        return jax.random.permutation(self._next(), n)
kernel_name = 'adaLN_cond__compressed_kv_cla__glu_gated_geglu__decode'

def setup_inputs():
    _rng = _Rng(jax.random.key(int.from_bytes(__import__("os").urandom(4), "little")))
    _w = lambda a: (lambda t: t.astype(jnp.bfloat16) if jnp.issubdtype(t.dtype, jnp.floating) else t)(jnp.asarray(a))

    def _A_setup():
        B, H, Sq, Sk, D, M = (1, 32, 1, 32768, 128, 512)
        Dc = 4 * D
        return {'x': _w((lambda *s: _rng.normal(s) * 0.05)(B, Sq, M)), 'c_kv': _w((lambda *s: _rng.normal(s) * 0.05)(B, Sk, Dc)), 'w_q': _w((lambda *s: _rng.normal(s) * 0.05)(M, H, D) * M ** (-0.5)), 'w_uk': _w((lambda *s: _rng.normal(s) * 0.05)(Dc, H, D) * Dc ** (-0.5)), 'w_uv': _w((lambda *s: _rng.normal(s) * 0.05)(Dc, H, D) * Dc ** (-0.5)), 'w_o': _w((lambda *s: _rng.normal(s) * 0.05)(H, D, M) * (H * D) ** (-0.5))}
    _A_in = _A_setup()

    def _B_setup():
        B, S, Dm, Df = (1, 1, 512, 1792)
        return {'x': _w((lambda *s: _rng.normal(s) * 0.05)(B, S, Dm)), 'w_gate': _w((lambda *s: _rng.normal(s) * 0.05)(Dm, Df) * Dm ** (-0.5)), 'w_up': _w((lambda *s: _rng.normal(s) * 0.05)(Dm, Df) * Dm ** (-0.5)), 'w_down': _w((lambda *s: _rng.normal(s) * 0.05)(Df, Dm) * Df ** (-0.5))}
    _B_in = _B_setup()
    return {'A_x': _A_in['x'], 'A_c_kv': _A_in['c_kv'], 'A_w_q': _A_in['w_q'], 'A_w_uk': _A_in['w_uk'], 'A_w_uv': _A_in['w_uv'], 'A_w_o': _A_in['w_o'], 'B_x': _B_in['x'], 'B_w_gate': _B_in['w_gate'], 'B_w_up': _B_in['w_up'], 'B_w_down': _B_in['w_down'], 'c': _w((lambda *s: _rng.normal(s) * 0.05)(1, 512)), 'w_mod': _w((lambda *s: _rng.normal(s) * 0.05)(512, 6 * 512) * 512 ** (-0.5))}

def reference(A_x, A_c_kv, A_w_q, A_w_uk, A_w_uv, A_w_o, B_x, B_w_gate, B_w_up, B_w_down, c, w_mod):

    def _A_ref(x, c_kv, w_q, w_uk, w_uv, w_o):
        B, Sq, M = (x.shape[0], x.shape[1], x.shape[2])
        Sk = c_kv.shape[1]
        H, D = (w_q.shape[1], w_q.shape[2])
        q = jnp.einsum('bqm,mhd->bhqd', x, w_q)
        k = jnp.einsum('bkc,chd->bhkd', c_kv, w_uk)
        v = jnp.einsum('bkc,chd->bhkd', c_kv, w_uv)
        scores = jnp.einsum('bhqd,bhkd->bhqk', q, k) * D ** (-0.5)
        off = Sk - Sq
        qi = jnp.arange(Sq)[:, None]
        kj = jnp.arange(Sk)[None, :]
        cmask = kj <= qi + off
        scores = jnp.where(cmask[None, None], scores, -1000000000.0)
        p = _softmax(scores, axis=-1)
        ctx = jnp.einsum('bhqk,bhkd->bhqd', p, v)
        return jnp.einsum('bhqd,hdm->bqm', ctx, w_o)

    def _B_ref(x, w_gate, w_up, w_down):
        g = jnp.einsum('bsd,df->bsf', x, w_gate)
        u = jnp.einsum('bsd,df->bsf', x, w_up)
        h = _gelu(g) * u
        return jnp.einsum('bsf,fd->bsd', h, w_down)
    x = A_x
    mod = (_silu(c) @ w_mod).reshape(c.shape[0], 6, 1, -1)
    sa, ca, ga, sb, cb, gb = (mod[:, 0].copy(), mod[:, 1].copy(), mod[:, 2].copy(), mod[:, 3].copy(), mod[:, 4].copy(), mod[:, 5].copy())
    h = _layernorm(x, axis=-1) * (1 + ca) + sa
    x = x + ga * _A_ref(h, A_c_kv, A_w_q, A_w_uk, A_w_uv, A_w_o)
    h = _layernorm(x, axis=-1) * (1 + cb) + sb
    x = x + gb * _B_ref(h, B_w_gate, B_w_up, B_w_down)
    return x
```

```python
import jax
import jax.numpy as jnp
from jax import lax
import jax.experimental.pallas as pl
import jax.experimental.pallas.tpu as pltpu

F32 = jnp.float32
BF16 = jnp.bfloat16
_NT = (((1,), (1,)), ((), ()))


def _layernorm(x, eps=1e-5):
    m = jnp.mean(x, axis=-1, keepdims=True)
    d = x - m
    v = jnp.mean(d * d, axis=-1, keepdims=True)
    return d * lax.rsqrt(v + eps)


def _gelu_tanh(x):
    c0 = 0.7978845608028654
    return 0.5 * x * (1.0 + jnp.tanh(c0 * (x + 0.044715 * (x * x * x))))


@jax.jit
def pallas_adaLN_cond__compressed_kv_cla__glu_gated_geglu__decode_kernel(
    A_x: jax.Array,
    A_c_kv: jax.Array,
    A_w_q: jax.Array,
    A_w_uk: jax.Array,
    A_w_uv: jax.Array,
    A_w_o: jax.Array,
    B_x: jax.Array,
    B_w_gate: jax.Array,
    B_w_up: jax.Array,
    B_w_down: jax.Array,
    c: jax.Array,
    w_mod: jax.Array,
):
    del B_x
    _, _, M = A_x.shape
    _, Sk, Dc = A_c_kv.shape
    _, H, D = A_w_q.shape
    Df = B_w_gate.shape[1]
    assert A_x.shape == (1, 1, M) and A_c_kv.shape[0] == 1
    assert D == 128 and M % 128 == 0 and Dc % 128 == 0 and Df % 128 == 0 and H % 16 == 0

    KV_CH = 4096
    BK = 2048
    assert Sk % KV_CH == 0 and KV_CH % BK == 0
    n_kv = Sk // KV_CH
    wd_chunks = [Df - 512, 384, 128] if Df >= 1024 else [Df]
    wd_offs = [sum(wd_chunks[:i]) for i in range(len(wd_chunks))]
    n_wd = len(wd_chunks)

    S_X, S_C, S_MOD, S_Q, S_UK = 0, 1, 2, 3, 4
    S_KV = 5
    S_UV = S_KV + n_kv
    S_O, S_G, S_U = S_UV + 1, S_UV + 2, S_UV + 3
    S_D = S_UV + 4
    n_sem = S_D + n_wd
    scale = float(D) ** -0.5

    def kernel(x_hbm, ckv_hbm, wq_hbm, wuk_hbm, wuv_hbm, wo_hbm, wg_hbm, wu_hbm, wd_hbm,
               c_hbm, wmod_hbm, o_ref,
               x_v, c_v, wmod_v, wq_v, wuk_v, ckv_v, wuv_v, wo_v, wg_v, wu_v, wd_v,
               hb_v, qa_v, ctx_v, sems):
        def cp(src, dst, s):
            return pltpu.make_async_copy(src, dst, sems.at[s])

        def kv_copy(i):
            rows = pl.ds(pl.multiple_of(i * KV_CH, KV_CH), KV_CH)
            return cp(ckv_hbm.at[0, rows, :], ckv_v.at[rows, :], S_KV + i)

        cp_x = cp(x_hbm, x_v, S_X)
        cp_c = cp(c_hbm, c_v, S_C)
        cp_mod = cp(wmod_hbm, wmod_v, S_MOD)
        cp_q = cp(wq_hbm, wq_v, S_Q)
        cp_uk = cp(wuk_hbm, wuk_v, S_UK)
        cp_uv = cp(wuv_hbm, wuv_v, S_UV)
        cp_o = cp(wo_hbm, wo_v, S_O)
        cp_g = cp(wg_hbm, wg_v, S_G)
        cp_u = cp(wu_hbm, wu_v, S_U)
        cp_d = [cp(wd_hbm.at[pl.ds(o, n), :], wd_v.at[pl.ds(o, n), :], S_D + i)
                for i, (o, n) in enumerate(zip(wd_offs, wd_chunks))]

        cp_mod.start()
        cp_x.start()
        cp_c.start()
        cp_q.start()
        cp_uk.start()
        for i in range(n_kv):
            kv_copy(i).start()
        cp_uv.start()
        cp_o.start()
        cp_g.start()
        cp_u.start()
        for d in cp_d:
            d.start()

        cp_c.wait()
        cp_x.wait()
        cvec = jnp.broadcast_to(c_v[...].astype(F32), (8, M))
        sc = (cvec * jax.nn.sigmoid(cvec)).astype(BF16)
        x0 = jnp.broadcast_to(x_v[0].astype(F32), (8, M))
        ln0 = _layernorm(x0)
        cp_mod.wait()
        mod = jnp.dot(sc, wmod_v[...], preferred_element_type=F32)
        sa, ca, ga, sb, cb, gb = (mod[:, i * M:(i + 1) * M] for i in range(6))
        h0 = ln0 * (1.0 + ca) + sa
        hb_v[...] = jnp.broadcast_to(h0[0:1, :], (128, M)).T

        cp_q.wait()
        UN = 16

        def q_body(i, acc):
            base = pl.multiple_of(i * UN, UN)
            for j in range(UN):
                acc = acc + hb_v[pl.ds(base + j, 1), :] * wq_v[base + j].astype(F32)
            return acc

        q = lax.fori_loop(0, M // UN, q_body, jnp.zeros((H, D), F32))
        q = q * scale

        cp_uk.wait()
        lane = lax.broadcasted_iota(jnp.int32, (H, 128), 1)

        def qa_body(cb_i, _):
            base = pl.multiple_of(cb_i * 128, 128)
            acc = jnp.zeros((H, 128), F32)
            for j in range(128):
                col = jnp.sum(q * wuk_v[base + j].astype(F32), axis=1, keepdims=True)
                acc = jnp.where(lane == j, col, acc)
            qa_v[cb_i] = acc
            return 0

        lax.fori_loop(0, Dc // 128, qa_body, 0)
        qa = jnp.concatenate([qa_v[i] for i in range(Dc // 128)], axis=1).astype(BF16)

        def kv_body(i, carry):
            kv_copy(i).wait()

            def blk(j, carry):
                m, l, acc = carry
                off = pl.multiple_of(i * KV_CH + j * BK, BK)
                kv = ckv_v[pl.ds(off, BK), :]
                s = lax.dot_general(qa, kv, _NT, preferred_element_type=F32)
                mn = jnp.maximum(m, jnp.max(s, axis=1, keepdims=True))
                a = jnp.exp(m - mn)
                p = jnp.exp(s - mn)
                l = a * l + jnp.sum(p, axis=1, keepdims=True)
                acc = a * acc + jnp.dot(p.astype(BF16), kv, preferred_element_type=F32)
                return mn, l, acc

            return lax.fori_loop(0, KV_CH // BK, blk, carry)

        init = (jnp.full((H, 1), -1e30, F32), jnp.zeros((H, 1), F32), jnp.zeros((H, Dc), F32))
        _, l_fin, acc_fin = lax.fori_loop(0, n_kv, kv_body, init)
        ctxc = acc_fin / l_fin
        for i in range(Dc // 128):
            qa_v[i] = ctxc[:, i * 128:(i + 1) * 128]

        cp_uv.wait()

        def ctx_body(cb_i, acc):
            base = pl.multiple_of(cb_i * 128, 128)
            blkv = qa_v[cb_i]
            for j in range(128):
                acc = acc + blkv[:, j:j + 1] * wuv_v[base + j].astype(F32)
            return acc

        ctx = lax.fori_loop(0, Dc // 128, ctx_body, jnp.zeros((H, D), F32))
        ctx_v[...] = ctx
        ctx_row = jnp.concatenate([ctx_v[h:h + 1, :] for h in range(H)], axis=1)
        ctx_row = jnp.broadcast_to(ctx_row, (8, H * D)).astype(BF16)

        cp_o.wait()
        attn = jnp.dot(ctx_row, wo_v[...].reshape(H * D, M), preferred_element_type=F32)
        x1 = x0 + ga * attn
        h1 = (_layernorm(x1) * (1.0 + cb) + sb).astype(BF16)

        cp_g.wait()
        g = jnp.dot(h1, wg_v[...], preferred_element_type=F32)
        cp_u.wait()
        u = jnp.dot(h1, wu_v[...], preferred_element_type=F32)
        hid = (_gelu_tanh(g) * u).astype(BF16)
        y = jnp.zeros((8, M), F32)
        for d, o, n in zip(cp_d, wd_offs, wd_chunks):
            d.wait()
            y = y + jnp.dot(hid[:, o:o + n], wd_v[o:o + n, :], preferred_element_type=F32)
        out = x1 + gb * y
        o_ref[0] = out[0:1, :].astype(o_ref.dtype)

    any_spec = pl.BlockSpec(memory_space=pl.ANY)
    return pl.pallas_call(
        kernel,
        out_shape=jax.ShapeDtypeStruct(A_x.shape, A_x.dtype),
        in_specs=[any_spec] * 11,
        out_specs=pl.BlockSpec(memory_space=pltpu.VMEM),
        scratch_shapes=[
            pltpu.VMEM(A_x.shape, A_x.dtype),
            pltpu.VMEM(c.shape, c.dtype),
            pltpu.VMEM(w_mod.shape, w_mod.dtype),
            pltpu.VMEM(A_w_q.shape, A_w_q.dtype),
            pltpu.VMEM(A_w_uk.shape, A_w_uk.dtype),
            pltpu.VMEM((Sk, Dc), A_c_kv.dtype),
            pltpu.VMEM(A_w_uv.shape, A_w_uv.dtype),
            pltpu.VMEM(A_w_o.shape, A_w_o.dtype),
            pltpu.VMEM(B_w_gate.shape, B_w_gate.dtype),
            pltpu.VMEM(B_w_up.shape, B_w_up.dtype),
            pltpu.VMEM(B_w_down.shape, B_w_down.dtype),
            pltpu.VMEM((M, 128), F32),
            pltpu.VMEM((Dc // 128, H, 128), F32),
            pltpu.VMEM((H, D), F32),
            pltpu.SemaphoreType.DMA((n_sem,)),
        ],
        compiler_params=pltpu.CompilerParams(vmem_limit_bytes=100 * 1024 * 1024),
    )(A_x, A_c_kv, A_w_q, A_w_uk, A_w_uv, A_w_o, B_w_gate, B_w_up, B_w_down, c, w_mod)
```

```python
import jax
import jax.numpy as jnp
from jax import lax
import jax.experimental.pallas as pl
import jax.experimental.pallas.tpu as pltpu

F32 = jnp.float32
BF16 = jnp.bfloat16
_NT = (((1,), (1,)), ((), ()))


def _layernorm(x, eps=1e-5):
    m = jnp.mean(x, axis=-1, keepdims=True)
    d = x - m
    v = jnp.mean(d * d, axis=-1, keepdims=True)
    return d * lax.rsqrt(v + eps)


def _gelu_tanh(x):
    c0 = 0.7978845608028654
    return 0.5 * x * (1.0 + jnp.tanh(c0 * (x + 0.044715 * (x * x * x))))


@jax.jit
def pallas_adaLN_cond__compressed_kv_cla__glu_gated_geglu__decode_kernel(
    A_x: jax.Array,
    A_c_kv: jax.Array,
    A_w_q: jax.Array,
    A_w_uk: jax.Array,
    A_w_uv: jax.Array,
    A_w_o: jax.Array,
    B_x: jax.Array,
    B_w_gate: jax.Array,
    B_w_up: jax.Array,
    B_w_down: jax.Array,
    c: jax.Array,
    w_mod: jax.Array,
):
    del B_x
    _, _, M = A_x.shape
    _, Sk, Dc = A_c_kv.shape
    _, H, D = A_w_q.shape
    Df = B_w_gate.shape[1]
    assert A_x.shape == (1, 1, M) and A_c_kv.shape[0] == 1
    assert D == 128 and M % 128 == 0 and Dc % 128 == 0 and Df % 128 == 0 and H % 16 == 0

    KV_CH = 8192
    BK = 2048
    assert Sk % KV_CH == 0 and KV_CH % BK == 0
    n_kv = Sk // KV_CH
    wd_chunks = [512, 512, 384, 256, 128]
    wd_offs = [sum(wd_chunks[:i]) for i in range(len(wd_chunks))]
    n_wd = len(wd_chunks)

    S_X, S_C, S_MOD, S_Q, S_UK = 0, 1, 2, 3, 4
    S_KV = 5
    S_UV = S_KV + n_kv
    S_O, S_G, S_U = S_UV + 1, S_UV + 2, S_UV + 3
    S_D = S_UV + 4
    n_sem = S_D + n_wd
    scale = float(D) ** -0.5

    def kernel(x_hbm, ckv_hbm, wq_hbm, wuk_hbm, wuv_hbm, wo_hbm, wg_hbm, wu_hbm, wd_hbm,
               c_hbm, wmod_hbm, o_ref,
               x_v, c_v, wmod_v, wq_v, wuk_v, ckv_v, wuv_v, wo_v, wg_v, wu_v, wd_v,
               hb_v, qa_v, ctx_v):
        pl.run_scoped(
            lambda sems: body(x_hbm, ckv_hbm, wq_hbm, wuk_hbm, wuv_hbm, wo_hbm, wg_hbm, wu_hbm,
                              wd_hbm, c_hbm, wmod_hbm, o_ref, x_v, c_v, wmod_v, wq_v, wuk_v,
                              ckv_v, wuv_v, wo_v, wg_v, wu_v, wd_v, hb_v, qa_v, ctx_v, sems),
            pltpu.SemaphoreType.DMA((n_sem,)))

    def body(x_hbm, ckv_hbm, wq_hbm, wuk_hbm, wuv_hbm, wo_hbm, wg_hbm, wu_hbm, wd_hbm,
             c_hbm, wmod_hbm, o_ref,
             x_v, c_v, wmod_v, wq_v, wuk_v, ckv_v, wuv_v, wo_v, wg_v, wu_v, wd_v,
             hb_v, qa_v, ctx_v, sems):
        def cp(src, dst, s):
            return pltpu.make_async_copy(src, dst, sems.at[s])

        def kv_copy(i):
            rows = pl.ds(pl.multiple_of(i * KV_CH, KV_CH), KV_CH)
            return cp(ckv_hbm.at[0, rows, :], ckv_v.at[rows, :], S_KV + i)

        cp_x = cp(x_hbm, x_v, S_X)
        cp_c = cp(c_hbm, c_v, S_C)
        cp_mod = cp(wmod_hbm, wmod_v, S_MOD)
        cp_q = cp(wq_hbm, wq_v, S_Q)
        cp_uk = cp(wuk_hbm, wuk_v, S_UK)
        cp_uv = cp(wuv_hbm, wuv_v, S_UV)
        cp_o = cp(wo_hbm, wo_v, S_O)
        cp_g = cp(wg_hbm, wg_v, S_G)
        cp_u = cp(wu_hbm, wu_v, S_U)
        cp_d = [cp(wd_hbm.at[pl.ds(o, n), :], wd_v.at[pl.ds(o, n), :], S_D + i)
                for i, (o, n) in enumerate(zip(wd_offs, wd_chunks))]

        cp_mod.start()
        cp_x.start()
        cp_c.start()
        cp_q.start()
        cp_uk.start()
        for i in range(n_kv):
            kv_copy(i).start()
        cp_uv.start()
        cp_o.start()
        cp_g.start()
        cp_u.start()
        for d in cp_d:
            d.start()

        cp_c.wait()
        cp_x.wait()
        cvec = jnp.broadcast_to(c_v[...].astype(F32), (8, M))
        sc = (cvec * jax.nn.sigmoid(cvec)).astype(BF16)
        x0 = jnp.broadcast_to(x_v[0].astype(F32), (8, M))
        ln0 = _layernorm(x0)
        cp_mod.wait()
        mod = jnp.dot(sc, wmod_v[...], preferred_element_type=F32)
        sa, ca, ga, sb, cb, gb = (mod[:, i * M:(i + 1) * M] for i in range(6))
        h0 = ln0 * (1.0 + ca) + sa
        hb_v[...] = jnp.broadcast_to(h0[0:1, :], (128, M)).T

        cp_q.wait()
        UN = 16

        def q_body(i, acc):
            base = pl.multiple_of(i * UN, UN)
            for j in range(UN):
                acc = acc + hb_v[pl.ds(base + j, 1), :] * wq_v[base + j].astype(F32)
            return acc

        q = lax.fori_loop(0, M // UN, q_body, jnp.zeros((H, D), F32))
        q = q * scale

        cp_uk.wait()
        lane = lax.broadcasted_iota(jnp.int32, (H, 128), 1)

        def qa_body(cb_i, _):
            base = pl.multiple_of(cb_i * 128, 128)
            acc = jnp.zeros((H, 128), F32)
            for j in range(128):
                col = jnp.sum(q * wuk_v[base + j].astype(F32), axis=1, keepdims=True)
                acc = jnp.where(lane == j, col, acc)
            qa_v[cb_i] = acc
            return 0

        lax.fori_loop(0, Dc // 128, qa_body, 0)
        qa = jnp.concatenate([qa_v[i] for i in range(Dc // 128)], axis=1).astype(BF16)

        def kv_body(i, carry):
            kv_copy(i).wait()

            def blk(j, carry):
                m, l, acc = carry
                off = pl.multiple_of(i * KV_CH + j * BK, BK)
                kv = ckv_v[pl.ds(off, BK), :]
                s = lax.dot_general(qa, kv, _NT, preferred_element_type=F32)
                mn = jnp.maximum(m, jnp.max(s, axis=1, keepdims=True))
                a = jnp.exp(m - mn)
                p = jnp.exp(s - mn)
                l = a * l + jnp.sum(p, axis=1, keepdims=True)
                acc = a * acc + jnp.dot(p.astype(BF16), kv, preferred_element_type=F32)
                return mn, l, acc

            return lax.fori_loop(0, KV_CH // BK, blk, carry)

        init = (jnp.full((H, 1), -1e30, F32), jnp.zeros((H, 1), F32), jnp.zeros((H, Dc), F32))
        _, l_fin, acc_fin = lax.fori_loop(0, n_kv, kv_body, init)
        ctxc = acc_fin / l_fin
        for i in range(Dc // 128):
            qa_v[i] = ctxc[:, i * 128:(i + 1) * 128]

        cp_uv.wait()

        def ctx_body(cb_i, acc):
            base = pl.multiple_of(cb_i * 128, 128)
            blkv = qa_v[cb_i]
            for j in range(128):
                acc = acc + blkv[:, j:j + 1] * wuv_v[base + j].astype(F32)
            return acc

        ctx = lax.fori_loop(0, Dc // 128, ctx_body, jnp.zeros((H, D), F32))
        ctx_v[...] = ctx
        ctx_row = jnp.concatenate([ctx_v[h:h + 1, :] for h in range(H)], axis=1)
        ctx_row = jnp.broadcast_to(ctx_row, (8, H * D)).astype(BF16)

        cp_o.wait()
        attn = jnp.dot(ctx_row, wo_v[...].reshape(H * D, M), preferred_element_type=F32)
        x1 = x0 + ga * attn
        h1 = (_layernorm(x1) * (1.0 + cb) + sb).astype(BF16)

        cp_g.wait()
        g = jnp.dot(h1, wg_v[...], preferred_element_type=F32)
        cp_u.wait()
        u = jnp.dot(h1, wu_v[...], preferred_element_type=F32)
        hid = (_gelu_tanh(g) * u).astype(BF16)
        y = jnp.zeros((8, M), F32)
        for d, o, n in zip(cp_d, wd_offs, wd_chunks):
            d.wait()
            y = y + jnp.dot(hid[:, o:o + n], wd_v[o:o + n, :], preferred_element_type=F32)
        out = x1 + gb * y
        o_ref[0] = out[0:1, :].astype(o_ref.dtype)

    any_spec = pl.BlockSpec(memory_space=pl.ANY)
    return pl.pallas_call(
        kernel,
        out_shape=jax.ShapeDtypeStruct(A_x.shape, A_x.dtype),
        in_specs=[any_spec] * 11,
        out_specs=pl.BlockSpec(memory_space=pltpu.VMEM),
        scratch_shapes=[
            pltpu.VMEM(A_x.shape, A_x.dtype),
            pltpu.VMEM(c.shape, c.dtype),
            pltpu.VMEM(w_mod.shape, w_mod.dtype),
            pltpu.VMEM(A_w_q.shape, A_w_q.dtype),
            pltpu.VMEM(A_w_uk.shape, A_w_uk.dtype),
            pltpu.VMEM((Sk, Dc), A_c_kv.dtype),
            pltpu.VMEM(A_w_uv.shape, A_w_uv.dtype),
            pltpu.VMEM(A_w_o.shape, A_w_o.dtype),
            pltpu.VMEM(B_w_gate.shape, B_w_gate.dtype),
            pltpu.VMEM(B_w_up.shape, B_w_up.dtype),
            pltpu.VMEM(B_w_down.shape, B_w_down.dtype),
            pltpu.VMEM((M, 128), F32),
            pltpu.VMEM((Dc // 128, H, 128), F32),
            pltpu.VMEM((H, D), F32),
        ],
        compiler_params=pltpu.CompilerParams(vmem_limit_bytes=100 * 1024 * 1024),
    )(A_x, A_c_kv, A_w_q, A_w_uk, A_w_uv, A_w_o, B_w_gate, B_w_up, B_w_down, c, w_mod)
```

```python
import jax
import jax.numpy as jnp
from jax import lax
import jax.experimental.pallas as pl
import jax.experimental.pallas.tpu as pltpu

F32 = jnp.float32
BF16 = jnp.bfloat16
_NT = (((1,), (1,)), ((), ()))


def _layernorm(x, eps=1e-5):
    m = jnp.mean(x, axis=-1, keepdims=True)
    d = x - m
    v = jnp.mean(d * d, axis=-1, keepdims=True)
    return d * lax.rsqrt(v + eps)


def _gelu_tanh(x):
    c0 = 0.7978845608028654
    return 0.5 * x * (1.0 + jnp.tanh(c0 * (x + 0.044715 * (x * x * x))))


@jax.jit
def pallas_adaLN_cond__compressed_kv_cla__glu_gated_geglu__decode_kernel(
    A_x: jax.Array,
    A_c_kv: jax.Array,
    A_w_q: jax.Array,
    A_w_uk: jax.Array,
    A_w_uv: jax.Array,
    A_w_o: jax.Array,
    B_x: jax.Array,
    B_w_gate: jax.Array,
    B_w_up: jax.Array,
    B_w_down: jax.Array,
    c: jax.Array,
    w_mod: jax.Array,
):
    del B_x
    _, _, M = A_x.shape
    _, Sk, Dc = A_c_kv.shape
    _, H, D = A_w_q.shape
    Df = B_w_gate.shape[1]
    assert A_x.shape == (1, 1, M) and A_c_kv.shape[0] == 1
    assert D == 128 and M % 128 == 0 and Dc % 128 == 0 and Df % 128 == 0 and H % 16 == 0

    KV_CH = 8192
    BK = 2048
    assert Sk % KV_CH == 0 and KV_CH % BK == 0
    n_kv = Sk // KV_CH
    wd_chunks = [512, 512, 384, 256]
    wv_chunks = [64, 32, 16, 16]
    wv_rows = sum(wv_chunks)
    assert sum(wd_chunks) + wv_rows == Df and wv_rows % 128 == 0
    assert all(n % 128 == 0 for n in wd_chunks) and all(n % 16 == 0 for n in wv_chunks)
    all_chunks = list(wd_chunks) + list(wv_chunks)
    all_offs = [sum(all_chunks[:i]) for i in range(len(all_chunks))]
    n_wd = len(all_chunks)
    n_mxu = len(wd_chunks)

    S_X, S_C, S_MOD, S_Q, S_UK = 0, 1, 2, 3, 4
    S_KV = 5
    S_UV = S_KV + n_kv
    S_O, S_G, S_U = S_UV + 1, S_UV + 2, S_UV + 3
    S_D = S_UV + 4
    n_sem = S_D + n_wd
    scale = float(D) ** -0.5

    def kernel(x_hbm, ckv_hbm, wq_hbm, wuk_hbm, wuv_hbm, wo_hbm, wg_hbm, wu_hbm, wd_hbm,
               c_hbm, wmod_hbm, o_ref,
               x_v, c_v, wmod_v, wq_v, wuk_v, ckv_v, wuv_v, wo_v, wg_v, wu_v, wd_v,
               hb_v, qa_v, ctx_v):
        pl.run_scoped(
            lambda sems: body(x_hbm, ckv_hbm, wq_hbm, wuk_hbm, wuv_hbm, wo_hbm, wg_hbm, wu_hbm,
                              wd_hbm, c_hbm, wmod_hbm, o_ref, x_v, c_v, wmod_v, wq_v, wuk_v,
                              ckv_v, wuv_v, wo_v, wg_v, wu_v, wd_v, hb_v, qa_v, ctx_v, sems),
            pltpu.SemaphoreType.DMA((n_sem,)))

    def body(x_hbm, ckv_hbm, wq_hbm, wuk_hbm, wuv_hbm, wo_hbm, wg_hbm, wu_hbm, wd_hbm,
             c_hbm, wmod_hbm, o_ref,
             x_v, c_v, wmod_v, wq_v, wuk_v, ckv_v, wuv_v, wo_v, wg_v, wu_v, wd_v,
             hb_v, qa_v, ctx_v, sems):
        def cp(src, dst, s):
            return pltpu.make_async_copy(src, dst, sems.at[s])

        def kv_copy(i):
            rows = pl.ds(pl.multiple_of(i * KV_CH, KV_CH), KV_CH)
            return cp(ckv_hbm.at[0, rows, :], ckv_v.at[rows, :], S_KV + i)

        cp_x = cp(x_hbm, x_v, S_X)
        cp_c = cp(c_hbm, c_v, S_C)
        cp_mod = cp(wmod_hbm, wmod_v, S_MOD)
        cp_q = cp(wq_hbm, wq_v, S_Q)
        cp_uk = cp(wuk_hbm, wuk_v, S_UK)
        cp_uv = cp(wuv_hbm, wuv_v, S_UV)
        cp_o = cp(wo_hbm, wo_v, S_O)
        cp_g = cp(wg_hbm, wg_v, S_G)
        cp_u = cp(wu_hbm, wu_v, S_U)
        cp_d = [cp(wd_hbm.at[pl.ds(o, n), :], wd_v.at[pl.ds(o, n), :], S_D + i)
                for i, (o, n) in enumerate(zip(all_offs, all_chunks))]

        cp_mod.start()
        cp_x.start()
        cp_c.start()
        cp_q.start()
        cp_uk.start()
        for i in range(n_kv):
            kv_copy(i).start()
        cp_uv.start()
        cp_o.start()
        cp_g.start()
        cp_u.start()
        for d in cp_d:
            d.start()

        cp_c.wait()
        cp_x.wait()
        cvec = jnp.broadcast_to(c_v[...].astype(F32), (8, M))
        sc = (cvec * jax.nn.sigmoid(cvec)).astype(BF16)
        x0 = jnp.broadcast_to(x_v[0].astype(F32), (8, M))
        ln0 = _layernorm(x0)
        cp_mod.wait()
        mod = jnp.dot(sc, wmod_v[...], preferred_element_type=F32)
        sa, ca, ga, sb, cb, gb = (mod[:, i * M:(i + 1) * M] for i in range(6))
        h0 = ln0 * (1.0 + ca) + sa
        hb_v[...] = jnp.broadcast_to(h0[0:1, :], (128, M)).T

        cp_q.wait()
        UN = 16

        def q_body(i, acc):
            base = pl.multiple_of(i * UN, UN)
            for j in range(UN):
                acc = acc + hb_v[pl.ds(base + j, 1), :] * wq_v[base + j].astype(F32)
            return acc

        q = lax.fori_loop(0, M // UN, q_body, jnp.zeros((H, D), F32))
        q = q * scale

        cp_uk.wait()
        lane = lax.broadcasted_iota(jnp.int32, (H, 128), 1)

        def qa_body(cb_i, _):
            base = pl.multiple_of(cb_i * 128, 128)
            acc = jnp.zeros((H, 128), F32)
            for j in range(128):
                col = jnp.sum(q * wuk_v[base + j].astype(F32), axis=1, keepdims=True)
                acc = jnp.where(lane == j, col, acc)
            qa_v[cb_i] = acc
            return 0

        lax.fori_loop(0, Dc // 128, qa_body, 0)
        qa = jnp.concatenate([qa_v[i] for i in range(Dc // 128)], axis=1).astype(BF16)

        def kv_body(i, carry):
            kv_copy(i).wait()

            def blk(j, carry):
                m, l, acc = carry
                off = pl.multiple_of(i * KV_CH + j * BK, BK)
                kv = ckv_v[pl.ds(off, BK), :]
                s = lax.dot_general(qa, kv, _NT, preferred_element_type=F32)
                mn = jnp.maximum(m, jnp.max(s, axis=1, keepdims=True))
                a = jnp.exp(m - mn)
                p = jnp.exp(s - mn)
                l = a * l + jnp.sum(p, axis=1, keepdims=True)
                acc = a * acc + jnp.dot(p.astype(BF16), kv, preferred_element_type=F32)
                return mn, l, acc

            return lax.fori_loop(0, KV_CH // BK, blk, carry)

        init = (jnp.full((H, 1), -1e30, F32), jnp.zeros((H, 1), F32), jnp.zeros((H, Dc), F32))
        _, l_fin, acc_fin = lax.fori_loop(0, n_kv, kv_body, init)
        ctxc = acc_fin / l_fin
        for i in range(Dc // 128):
            qa_v[i] = ctxc[:, i * 128:(i + 1) * 128]

        cp_uv.wait()

        def ctx_body(cb_i, acc):
            base = pl.multiple_of(cb_i * 128, 128)
            blkv = qa_v[cb_i]
            for j in range(128):
                acc = acc + blkv[:, j:j + 1] * wuv_v[base + j].astype(F32)
            return acc

        ctx = lax.fori_loop(0, Dc // 128, ctx_body, jnp.zeros((H, D), F32))
        ctx_v[...] = ctx
        ctx_row = jnp.concatenate([ctx_v[h:h + 1, :] for h in range(H)], axis=1)
        ctx_row = jnp.broadcast_to(ctx_row, (8, H * D)).astype(BF16)

        cp_o.wait()
        attn = jnp.dot(ctx_row, wo_v[...].reshape(H * D, M), preferred_element_type=F32)
        x1 = x0 + ga * attn
        h1 = (_layernorm(x1) * (1.0 + cb) + sb).astype(BF16)

        cp_g.wait()
        g = jnp.dot(h1, wg_v[...], preferred_element_type=F32)
        cp_u.wait()
        u = jnp.dot(h1, wu_v[...], preferred_element_type=F32)
        hid = (_gelu_tanh(g) * u).astype(BF16)
        f0 = Df - wv_rows
        hm = jnp.broadcast_to(hid[0:1, f0:].astype(F32), (128, wv_rows)).T
        y = jnp.zeros((8, M), F32)
        for i in range(n_mxu):
            o, n = all_offs[i], all_chunks[i]
            cp_d[i].wait()
            y = y + jnp.dot(hid[:, o:o + n], wd_v[o:o + n, :], preferred_element_type=F32)
        row = lax.broadcasted_iota(jnp.int32, (8, M), 0)
        acc = jnp.where(row == 0, y, 0.0)
        for i in range(n_mxu, n_wd):
            o, n = all_offs[i], all_chunks[i]
            cp_d[i].wait()
            for r in range(o, o + n, 8):
                if r % 16 == 0:
                    wt = wd_v[r:r + 16, :].astype(F32)
                    w8 = wt[0:8]
                else:
                    w8 = wt[8:16]
                mul = hm[r - f0:r - f0 + 8, :]
                acc = acc + w8 * jnp.concatenate([mul] * (M // 128), axis=1)
        out = x1[0:1] + gb[0:1] * jnp.sum(acc, axis=0, keepdims=True)
        o_ref[0] = out.astype(o_ref.dtype)

    any_spec = pl.BlockSpec(memory_space=pl.ANY)
    return pl.pallas_call(
        kernel,
        out_shape=jax.ShapeDtypeStruct(A_x.shape, A_x.dtype),
        in_specs=[any_spec] * 11,
        out_specs=pl.BlockSpec(memory_space=pltpu.VMEM),
        scratch_shapes=[
            pltpu.VMEM(A_x.shape, A_x.dtype),
            pltpu.VMEM(c.shape, c.dtype),
            pltpu.VMEM(w_mod.shape, w_mod.dtype),
            pltpu.VMEM(A_w_q.shape, A_w_q.dtype),
            pltpu.VMEM(A_w_uk.shape, A_w_uk.dtype),
            pltpu.VMEM((Sk, Dc), A_c_kv.dtype),
            pltpu.VMEM(A_w_uv.shape, A_w_uv.dtype),
            pltpu.VMEM(A_w_o.shape, A_w_o.dtype),
            pltpu.VMEM(B_w_gate.shape, B_w_gate.dtype),
            pltpu.VMEM(B_w_up.shape, B_w_up.dtype),
            pltpu.VMEM(B_w_down.shape, B_w_down.dtype),
            pltpu.VMEM((M, 128), F32),
            pltpu.VMEM((Dc // 128, H, 128), F32),
            pltpu.VMEM((H, D), F32),
        ],
        compiler_params=pltpu.CompilerParams(vmem_limit_bytes=100 * 1024 * 1024),
    )(A_x, A_c_kv, A_w_q, A_w_uk, A_w_uv, A_w_o, B_w_gate, B_w_up, B_w_down, c, w_mod)
```

```python
import jax
import jax.numpy as jnp
from jax import lax
import jax.experimental.pallas as pl
import jax.experimental.pallas.tpu as pltpu

F32 = jnp.float32
BF16 = jnp.bfloat16
_NT = (((1,), (1,)), ((), ()))


def _layernorm(x, eps=1e-5):
    m = jnp.mean(x, axis=-1, keepdims=True)
    d = x - m
    v = jnp.mean(d * d, axis=-1, keepdims=True)
    return d * lax.rsqrt(v + eps)


def _gelu_tanh(x):
    c0 = 0.7978845608028654
    return 0.5 * x * (1.0 + jnp.tanh(c0 * (x + 0.044715 * (x * x * x))))


@jax.jit
def pallas_adaLN_cond__compressed_kv_cla__glu_gated_geglu__decode_kernel(
    A_x: jax.Array,
    A_c_kv: jax.Array,
    A_w_q: jax.Array,
    A_w_uk: jax.Array,
    A_w_uv: jax.Array,
    A_w_o: jax.Array,
    B_x: jax.Array,
    B_w_gate: jax.Array,
    B_w_up: jax.Array,
    B_w_down: jax.Array,
    c: jax.Array,
    w_mod: jax.Array,
):
    del B_x
    _, _, M = A_x.shape
    _, Sk, Dc = A_c_kv.shape
    _, H, D = A_w_q.shape
    Df = B_w_gate.shape[1]
    assert A_x.shape == (1, 1, 512) and A_c_kv.shape[0] == 1 and Dc == 512
    assert (H, D) == (32, 128) and Df == 1792 and w_mod.shape == (M, 6 * M)

    BK = 1024
    NG = 4
    LOOK = NG
    n_kv = Sk // BK
    assert Sk % BK == 0 and n_kv >= LOOK
    KV_S = 8
    KV_R0 = 32
    KV_R1 = 32
    kv_steps = BK // (KV_S // 2 * (KV_R0 + KV_R1))
    kv_nstep = n_kv * kv_steps
    assert kv_steps * (KV_S // 2) * (KV_R0 + KV_R1) == BK
    WD_MXU = [512, 512, 256, 256]
    WD_VPU = [128, 64, 32, 16, 16]
    WD_PAT = [(0, 1), (0, 1), (1,), (1,)]
    wv_rows = sum(WD_VPU)
    assert sum(WD_MXU) + wv_rows == Df and wv_rows % 128 == 0
    assert all(n % 128 == 0 for n in WD_MXU) and all(n % 16 == 0 for n in WD_VPU)
    wd_chunks = list(WD_MXU) + list(WD_VPU)
    wd_offs = [sum(wd_chunks[:i]) for i in range(len(wd_chunks))]
    n_mxu, n_wd = len(WD_MXU), len(wd_chunks)

    S_X, S_C, S_MOD = 0, 1, 2
    S_Q = 3
    S_UK = S_Q + NG
    S_KV = S_UK + NG
    S_UV = S_KV + n_kv
    S_O = S_UV + NG
    S_GU = S_O + NG
    S_D = S_GU + NG
    n_sem = S_D + n_wd
    scale = float(D) ** -0.5

    def kernel(*refs):
        pl.run_scoped(lambda sems: body(*refs, sems), pltpu.SemaphoreType.DMA((n_sem,)))

    def body(x_hbm, ckv_hbm, wq_hbm, wuk_hbm, wuv_hbm, wo_hbm, wg_hbm, wu_hbm, wd_hbm,
             c_hbm, wmod_hbm, o_ref,
             x_v, c_v, wmod_v, wq_v, wuk_v, ckv_v, wuv_v, wo_v, wgu_v, wd_v,
             hb_v, qa_v, ctx_v, sems):

        def start(src, dst, s, prio):
            pltpu.make_async_copy(src, dst, sems.at[s]).start(priority=prio)

        def wait_filled(buf, s):
            pltpu.make_async_copy(buf, buf, sems.at[s]).wait()

        def loop(n, step):
            lax.fori_loop(0, n, lambda k, _: step(k) or 0, 0)

        def issue_mod():
            def step(k):
                band, third = k // 3, k % 3
                for j in range(4):
                    rows = pl.ds(pl.multiple_of((j * 8 + band) * 16, 16), 16)
                    cols = pl.ds(pl.multiple_of(third * 1024, 1024), 1024)
                    start(wmod_hbm.at[rows, cols], wmod_v.at[rows, cols], S_MOD, j % 2)
            loop(24, step)

        def issue_w3(hbm, vm, s0, g):
            def step(k):
                for j in range(4):
                    rows = pl.ds(g * 128 + j * 32 + k * 4, 4)
                    start(hbm.at[rows], vm.at[rows], s0 + g, j % 2)
            loop(8, step)

        def wait_w3(vm, s0, g):
            wait_filled(vm.at[pl.ds(g * 128, 128)], s0 + g)

        def issue_kv(b):
            def step(t):
                k = b * kv_steps + t
                for j in range(KV_S // 2):
                    for q, (r, base) in enumerate(((KV_R0, 0), (KV_R1, kv_nstep * KV_R0))):
                        src = (j * (KV_R0 + KV_R1) * kv_nstep + base) + k * r
                        dst = b * BK + (t * (KV_S // 2) + j) * (KV_R0 + KV_R1) + q * KV_R0
                        start(ckv_hbm.at[0, pl.ds(pl.multiple_of(src, 16), r), :],
                              ckv_v.at[pl.ds(pl.multiple_of(dst, 16), r), :], S_KV + b, q)
            loop(kv_steps, step)

        def issue_wo(g):
            def step(k):
                for j in range(4):
                    h = g * 8 + j * 2 + k // 4
                    rows = pl.ds(pl.multiple_of((k % 4) * 32, 32), 32)
                    start(wo_hbm.at[h, rows, :], wo_v.at[h, rows, :], S_O + g, j % 2)
            loop(8, step)

        def issue_gu(g):
            def step(k):
                rows = pl.ds(pl.multiple_of(g * 128 + k * 16, 16), 16)
                drows = pl.ds(pl.multiple_of(k * 16, 16), 16)
                for half in range(2):
                    cols = pl.ds(half * (Df // 2), Df // 2)
                    start(wg_hbm.at[rows, cols], wgu_v.at[g, 0, drows, cols], S_GU + g, 0)
                    start(wu_hbm.at[rows, cols], wgu_v.at[g, 1, drows, cols], S_GU + g, 1)
            loop(8, step)

        def issue_wd(i):
            o, n = wd_offs[i], wd_chunks[i]
            pat = WD_PAT[i] if i < n_mxu else (1,)
            piece = min(n, 32)
            npc = n // piece
            if npc <= 2 * len(pat):
                for k in range(npc):
                    rows = pl.ds(o + k * piece, piece)
                    start(wd_hbm.at[rows, :], wd_v.at[rows, :], S_D + i, pat[k % len(pat)])
                return

            def step(k):
                for j, prio in enumerate(pat):
                    rows = pl.ds(pl.multiple_of(o + (k * len(pat) + j) * piece, piece), piece)
                    start(wd_hbm.at[rows, :], wd_v.at[rows, :], S_D + i, prio)
            loop(npc // len(pat), step)

        wd_plan = [[0], [1], [2], list(range(3, n_wd))] if n_mxu >= 4 else [list(range(n_wd)), [], [], []]

        start(x_hbm, x_v, S_X, 0)
        start(c_hbm, c_v, S_C, 0)
        issue_mod()
        for g in range(LOOK):
            issue_w3(wq_hbm, wq_v, S_Q, g)

        wait_filled(c_v, S_C)
        wait_filled(x_v, S_X)
        cvec = jnp.broadcast_to(c_v[...].astype(F32), (8, M))
        sc = (cvec * jax.nn.sigmoid(cvec)).astype(BF16)
        x0 = jnp.broadcast_to(x_v[0].astype(F32), (8, M))
        ln0 = _layernorm(x0)
        wait_filled(wmod_v, S_MOD)
        mod = jnp.dot(sc, wmod_v[...], preferred_element_type=F32)
        sa, ca, ga, sb, cb, gb = (mod[:, i * M:(i + 1) * M] for i in range(6))
        h0 = ln0 * (1.0 + ca) + sa
        hb_v[...] = jnp.broadcast_to(h0[0:1, :], (128, M)).T

        def q_group(g, acc):
            issue_w3(wuk_hbm, wuk_v, S_UK, g)
            wait_w3(wq_v, S_Q, g)

            def q_part(i, acc):
                base = pl.multiple_of(g * 128 + i * 16, 16)
                for j in range(16):
                    acc = acc + hb_v[pl.ds(base + j, 1), :] * wq_v[base + j].astype(F32)
                return acc

            return lax.fori_loop(0, 8, q_part, acc)

        q = lax.fori_loop(0, NG, q_group, jnp.zeros((H, D), F32)) * scale

        lane = lax.broadcasted_iota(jnp.int32, (H, 128), 1)

        def qa_group(g, _):
            issue_kv(g)
            wait_w3(wuk_v, S_UK, g)
            base = pl.multiple_of(g * 128, 128)
            acc = jnp.zeros((H, 128), F32)
            for j in range(128):
                col = jnp.sum(q * wuk_v[base + j].astype(F32), axis=1, keepdims=True)
                acc = jnp.where(lane == j, col, acc)
            qa_v[g] = acc
            return 0

        lax.fori_loop(0, NG, qa_group, 0)
        qa = jnp.concatenate([qa_v[i] for i in range(NG)], axis=1).astype(BF16)

        def kv_group(b, carry):
            @pl.when(b + LOOK < n_kv)
            def _():
                issue_kv(b + LOOK)

            @pl.when(b + LOOK >= n_kv)
            def _():
                issue_w3(wuv_hbm, wuv_v, S_UV, b + LOOK - n_kv)

            rows = pl.ds(pl.multiple_of(b * BK, BK), BK)
            wait_filled(ckv_v.at[rows, :], S_KV + b)
            m, l, acc = carry
            kv = ckv_v[rows, :]
            s = lax.dot_general(qa, kv, _NT, preferred_element_type=F32)
            mn = jnp.maximum(m, jnp.max(s, axis=1, keepdims=True))
            a = jnp.exp(m - mn)
            p = jnp.exp(s - mn)
            l = a * l + jnp.sum(p, axis=1, keepdims=True)
            acc = a * acc + jnp.dot(p.astype(BF16), kv, preferred_element_type=F32)
            return mn, l, acc

        init = (jnp.full((H, 1), -jnp.inf, F32), jnp.zeros((H, 1), F32), jnp.zeros((H, Dc), F32))
        _, l_fin, acc_fin = lax.fori_loop(0, n_kv, kv_group, init)
        ctxc = acc_fin / l_fin
        for i in range(NG):
            qa_v[i] = ctxc[:, i * 128:(i + 1) * 128]

        def ctx_group(g, acc):
            issue_wo(g)
            wait_w3(wuv_v, S_UV, g)
            base = pl.multiple_of(g * 128, 128)
            blk = qa_v[g]
            for j in range(128):
                acc = acc + blk[:, j:j + 1] * wuv_v[base + j].astype(F32)
            return acc

        ctx_v[...] = lax.fori_loop(0, NG, ctx_group, jnp.zeros((H, D), F32))
        ctx_row = jnp.concatenate([ctx_v[h:h + 1, :] for h in range(H)], axis=1)
        ctx_row = jnp.broadcast_to(ctx_row, (8, H * D)).astype(BF16)

        attn = jnp.zeros((8, M), F32)
        for g in range(NG):
            issue_gu(g)
            wait_filled(wo_v.at[pl.ds(g * 8, 8)], S_O + g)
            wo_g = wo_v[g * 8:(g + 1) * 8].reshape(8 * D, M)
            attn = attn + jnp.dot(ctx_row[:, g * 8 * D:(g + 1) * 8 * D], wo_g,
                                  preferred_element_type=F32)
        x1 = x0 + ga * attn
        h1 = (_layernorm(x1) * (1.0 + cb) + sb).astype(BF16)

        gate = jnp.zeros((8, Df), F32)
        up = jnp.zeros((8, Df), F32)
        for g in range(NG):
            for i in wd_plan[g]:
                issue_wd(i)
            wait_filled(wgu_v.at[g], S_GU + g)
            hk = h1[:, g * 128:(g + 1) * 128]
            gate = gate + jnp.dot(hk, wgu_v[g, 0], preferred_element_type=F32)
            up = up + jnp.dot(hk, wgu_v[g, 1], preferred_element_type=F32)
        hid = (_gelu_tanh(gate) * up).astype(BF16)

        f0 = Df - wv_rows
        hm = jnp.broadcast_to(hid[0:1, f0:].astype(F32), (128, wv_rows)).T
        y = jnp.zeros((8, M), F32)
        for i in range(n_mxu):
            o, n = wd_offs[i], wd_chunks[i]
            wait_filled(wd_v.at[pl.ds(o, n), :], S_D + i)
            y = y + jnp.dot(hid[:, o:o + n], wd_v[o:o + n, :], preferred_element_type=F32)
        row = lax.broadcasted_iota(jnp.int32, (8, M), 0)
        acc = jnp.where(row == 0, y, 0.0)
        for i in range(n_mxu, n_wd):
            o, n = wd_offs[i], wd_chunks[i]
            wait_filled(wd_v.at[pl.ds(o, n), :], S_D + i)
            for r in range(o, o + n, 16):
                wt = wd_v[r:r + 16, :].astype(F32)
                for t in range(2):
                    mul = hm[r - f0 + 8 * t:r - f0 + 8 * t + 8, :]
                    acc = acc + wt[8 * t:8 * t + 8] * jnp.concatenate([mul] * (M // 128), axis=1)
        out = x1[0:1] + gb[0:1] * jnp.sum(acc, axis=0, keepdims=True)
        o_ref[0] = out.astype(o_ref.dtype)

    any_spec = pl.BlockSpec(memory_space=pl.ANY)
    return pl.pallas_call(
        kernel,
        out_shape=jax.ShapeDtypeStruct(A_x.shape, A_x.dtype),
        in_specs=[any_spec] * 11,
        out_specs=pl.BlockSpec(memory_space=pltpu.VMEM),
        scratch_shapes=[
            pltpu.VMEM(A_x.shape, A_x.dtype),
            pltpu.VMEM(c.shape, c.dtype),
            pltpu.VMEM(w_mod.shape, w_mod.dtype),
            pltpu.VMEM(A_w_q.shape, A_w_q.dtype),
            pltpu.VMEM(A_w_uk.shape, A_w_uk.dtype),
            pltpu.VMEM((Sk, Dc), A_c_kv.dtype),
            pltpu.VMEM(A_w_uv.shape, A_w_uv.dtype),
            pltpu.VMEM(A_w_o.shape, A_w_o.dtype),
            pltpu.VMEM((NG, 2, M // NG, Df), B_w_gate.dtype),
            pltpu.VMEM(B_w_down.shape, B_w_down.dtype),
            pltpu.VMEM((M, 128), F32),
            pltpu.VMEM((NG, H, 128), F32),
            pltpu.VMEM((H, D), F32),
        ],
        compiler_params=pltpu.CompilerParams(vmem_limit_bytes=100 * 1024 * 1024),
    )(A_x, A_c_kv, A_w_q, A_w_uk, A_w_uv, A_w_o, B_w_gate, B_w_up, B_w_down, c, w_mod)
```

```python
import jax
import jax.numpy as jnp
from jax import lax
import jax.experimental.pallas as pl
import jax.experimental.pallas.tpu as pltpu

F32 = jnp.float32
BF16 = jnp.bfloat16
_NT = (((1,), (1,)), ((), ()))


def _layernorm(x, eps=1e-5):
    m = jnp.mean(x, axis=-1, keepdims=True)
    d = x - m
    v = jnp.mean(d * d, axis=-1, keepdims=True)
    return d * lax.rsqrt(v + eps)


def _gelu_tanh(x):
    c0 = 0.7978845608028654
    return 0.5 * x * (1.0 + jnp.tanh(c0 * (x + 0.044715 * (x * x * x))))


@jax.jit
def pallas_adaLN_cond__compressed_kv_cla__glu_gated_geglu__decode_kernel(
    A_x: jax.Array,
    A_c_kv: jax.Array,
    A_w_q: jax.Array,
    A_w_uk: jax.Array,
    A_w_uv: jax.Array,
    A_w_o: jax.Array,
    B_x: jax.Array,
    B_w_gate: jax.Array,
    B_w_up: jax.Array,
    B_w_down: jax.Array,
    c: jax.Array,
    w_mod: jax.Array,
):
    del B_x
    _, _, M = A_x.shape
    _, Sk, Dc = A_c_kv.shape
    _, H, D = A_w_q.shape
    Df = B_w_gate.shape[1]
    assert A_x.shape == (1, 1, 512) and A_c_kv.shape[0] == 1 and Dc == 512
    assert (H, D) == (32, 128) and Df == 1792 and w_mod.shape == (M, 6 * M)

    BK = 1024
    NG = 4
    LOOK = NG
    n_kv = Sk // BK
    assert Sk % BK == 0 and n_kv >= LOOK
    KV_S = 8
    KV_R = 32
    KV_PAT = (0, 1)
    KV_UNROLL = 1
    KV_SPLIT = 0
    kv_steps = BK // (KV_S * KV_R)
    kv_nstep = n_kv * kv_steps
    assert kv_steps * KV_S * KV_R == BK
    W3_S = 4
    W3_PAT = (0, 1)
    W3_R = 4
    WO_S = 4
    WO_PAT = (0, 1)
    MOD_S = 4
    MOD_PAT = (0, 1)
    GU_PAT = (0, 1, 0, 1)
    WD_MXU = [512, 512, 256, 256]
    WD_VPU = [128, 64, 32, 16, 16]
    WD_PAT = [(0, 1), (0, 1), (1,), (1,)]
    wv_rows = sum(WD_VPU)
    assert sum(WD_MXU) + wv_rows == Df and wv_rows % 128 == 0
    assert all(n % 128 == 0 for n in WD_MXU) and all(n % 16 == 0 for n in WD_VPU)
    wd_chunks = list(WD_MXU) + list(WD_VPU)
    wd_offs = [sum(wd_chunks[:i]) for i in range(len(wd_chunks))]
    n_mxu, n_wd = len(WD_MXU), len(wd_chunks)

    S_X, S_C, S_MOD = 0, 1, 2
    S_Q = 3
    S_UK = S_Q + NG
    S_KV = S_UK + NG
    S_UV = S_KV + n_kv
    S_O = S_UV + NG
    S_GU = S_O + NG
    S_D = S_GU + NG
    n_sem = S_D + n_wd
    scale = float(D) ** -0.5

    def kernel(*refs):
        pl.run_scoped(lambda sems: body(*refs, sems), pltpu.SemaphoreType.DMA((n_sem,)))

    def body(x_hbm, ckv_hbm, wq_hbm, wuk_hbm, wuv_hbm, wo_hbm, wg_hbm, wu_hbm, wd_hbm,
             c_hbm, wmod_hbm, o_ref,
             x_v, c_v, wmod_v, wq_v, wuk_v, ckv_v, wuv_v, wo_v, wgu_v, wd_v,
             hb_v, qa_v, ctx_v, sems):

        def start(src, dst, s, prio):
            pltpu.make_async_copy(src, dst, sems.at[s]).start(priority=prio)

        def wait_filled(buf, s):
            pltpu.make_async_copy(buf, buf, sems.at[s]).wait()

        def loop(n, step):
            lax.fori_loop(0, n, lambda k, _: step(k) or 0, 0)

        def issue_mod():
            bands = 32 // MOD_S

            def step(band):
                for third in range(3):
                    for j in range(MOD_S):
                        rows = pl.ds(pl.multiple_of((j * bands + band) * 16, 16), 16)
                        cols = pl.ds(third * 1024, 1024)
                        start(wmod_hbm.at[rows, cols], wmod_v.at[rows, cols], S_MOD,
                              MOD_PAT[j % len(MOD_PAT)])
            loop(bands, step)

        def issue_w3(hbm, vm, s0, g):
            per = 128 // W3_S

            def step(k):
                for j in range(W3_S):
                    rows = pl.ds(g * 128 + j * per + k * W3_R, W3_R)
                    start(hbm.at[rows], vm.at[rows], s0 + g, W3_PAT[j % len(W3_PAT)])
            loop(per // W3_R, step)

        def wait_w3(vm, s0, g):
            wait_filled(vm.at[pl.ds(g * 128, 128)], s0 + g)

        def issue_kv(b, t0=0, t1=kv_steps):
            def step(t):
                k = b * kv_steps + t
                for j in range(KV_S):
                    src = (j * kv_nstep + k) * KV_R
                    dst = b * BK + (t * KV_S + j) * KV_R
                    start(ckv_hbm.at[0, pl.ds(pl.multiple_of(src, KV_R), KV_R), :],
                          ckv_v.at[pl.ds(pl.multiple_of(dst, KV_R), KV_R), :], S_KV + b,
                          KV_PAT[j % len(KV_PAT)])
            lax.fori_loop(t0, t1, lambda t, _: step(t) or 0, 0, unroll=KV_UNROLL)

        def issue_wo(g):
            hper = 8 // WO_S

            def step(hh):
                for part in range(4):
                    for j in range(WO_S):
                        h = g * 8 + j * hper + hh
                        rows = pl.ds(part * 32, 32)
                        start(wo_hbm.at[h, rows, :], wo_v.at[h, rows, :], S_O + g,
                              WO_PAT[j % len(WO_PAT)])
            loop(hper, step)

        def issue_gu(g):
            def step(k):
                rows = pl.ds(pl.multiple_of(g * 128 + k * 16, 16), 16)
                drows = pl.ds(pl.multiple_of(k * 16, 16), 16)
                for half in range(2):
                    cols = pl.ds(half * (Df // 2), Df // 2)
                    start(wg_hbm.at[rows, cols], wgu_v.at[g, 0, drows, cols], S_GU + g,
                          GU_PAT[2 * half])
                    start(wu_hbm.at[rows, cols], wgu_v.at[g, 1, drows, cols], S_GU + g,
                          GU_PAT[2 * half + 1])
            loop(8, step)

        def issue_wd(i):
            o, n = wd_offs[i], wd_chunks[i]
            pat = WD_PAT[i] if i < n_mxu else (1,)
            piece = min(n, 32)
            npc = n // piece
            if npc <= 2 * len(pat):
                for k in range(npc):
                    rows = pl.ds(o + k * piece, piece)
                    start(wd_hbm.at[rows, :], wd_v.at[rows, :], S_D + i, pat[k % len(pat)])
                return

            def step(k):
                for j, prio in enumerate(pat):
                    rows = pl.ds(pl.multiple_of(o + (k * len(pat) + j) * piece, piece), piece)
                    start(wd_hbm.at[rows, :], wd_v.at[rows, :], S_D + i, prio)
            loop(npc // len(pat), step)

        wd_plan = [[0], [1], [2], list(range(3, n_wd))] if n_mxu >= 4 else [list(range(n_wd)), [], [], []]

        start(x_hbm, x_v, S_X, 0)
        start(c_hbm, c_v, S_C, 0)
        issue_mod()
        for g in range(LOOK):
            issue_w3(wq_hbm, wq_v, S_Q, g)

        wait_filled(c_v, S_C)
        wait_filled(x_v, S_X)
        cvec = jnp.broadcast_to(c_v[...].astype(F32), (8, M))
        sc = (cvec * jax.nn.sigmoid(cvec)).astype(BF16)
        x0 = jnp.broadcast_to(x_v[0].astype(F32), (8, M))
        ln0 = _layernorm(x0)
        wait_filled(wmod_v, S_MOD)
        mod = jnp.dot(sc, wmod_v[...], preferred_element_type=F32)
        sa, ca, ga, sb, cb, gb = (mod[:, i * M:(i + 1) * M] for i in range(6))
        h0 = ln0 * (1.0 + ca) + sa
        hb_v[...] = jnp.broadcast_to(h0[0:1, :], (128, M)).T

        def q_group(g, acc):
            issue_w3(wuk_hbm, wuk_v, S_UK, g)
            wait_w3(wq_v, S_Q, g)

            def q_part(i, acc):
                base = pl.multiple_of(g * 128 + i * 16, 16)
                for j in range(16):
                    acc = acc + hb_v[pl.ds(base + j, 1), :] * wq_v[base + j].astype(F32)
                return acc

            return lax.fori_loop(0, 8, q_part, acc)

        q = lax.fori_loop(0, NG, q_group, jnp.zeros((H, D), F32)) * scale

        lane = lax.broadcasted_iota(jnp.int32, (H, 128), 1)

        def qa_group(g, _):
            issue_kv(g)
            wait_w3(wuk_v, S_UK, g)
            base = pl.multiple_of(g * 128, 128)
            acc = jnp.zeros((H, 128), F32)
            for j in range(128):
                col = jnp.sum(q * wuk_v[base + j].astype(F32), axis=1, keepdims=True)
                acc = jnp.where(lane == j, col, acc)
            qa_v[g] = acc
            return 0

        lax.fori_loop(0, NG, qa_group, 0)
        qa = jnp.concatenate([qa_v[i] for i in range(NG)], axis=1).astype(BF16)

        def kv_group(b, carry):
            @pl.when(b + LOOK < n_kv)
            def _():
                issue_kv(b + LOOK, 0, kv_steps - KV_SPLIT)

            @pl.when(b + LOOK >= n_kv)
            def _():
                issue_w3(wuv_hbm, wuv_v, S_UV, b + LOOK - n_kv)

            rows = pl.ds(pl.multiple_of(b * BK, BK), BK)
            wait_filled(ckv_v.at[rows, :], S_KV + b)
            m, l, acc = carry
            kv = ckv_v[rows, :]
            s = lax.dot_general(qa, kv, _NT, preferred_element_type=F32)
            mn = jnp.maximum(m, jnp.max(s, axis=1, keepdims=True))
            a = jnp.exp(m - mn)
            p = jnp.exp(s - mn)
            l = a * l + jnp.sum(p, axis=1, keepdims=True)
            if KV_SPLIT:
                @pl.when(b + LOOK < n_kv)
                def _():
                    issue_kv(b + LOOK, kv_steps - KV_SPLIT, kv_steps)
                kv = ckv_v[rows, :]
            acc = a * acc + jnp.dot(p.astype(BF16), kv, preferred_element_type=F32)
            return mn, l, acc

        init = (jnp.full((H, 1), -jnp.inf, F32), jnp.zeros((H, 1), F32), jnp.zeros((H, Dc), F32))
        _, l_fin, acc_fin = lax.fori_loop(0, n_kv, kv_group, init)
        ctxc = acc_fin / l_fin
        for i in range(NG):
            qa_v[i] = ctxc[:, i * 128:(i + 1) * 128]

        def ctx_group(g, acc):
            issue_wo(g)
            wait_w3(wuv_v, S_UV, g)
            base = pl.multiple_of(g * 128, 128)
            blk = qa_v[g]
            for j in range(128):
                acc = acc + blk[:, j:j + 1] * wuv_v[base + j].astype(F32)
            return acc

        ctx_v[...] = lax.fori_loop(0, NG, ctx_group, jnp.zeros((H, D), F32))
        ctx_row = jnp.concatenate([ctx_v[h:h + 1, :] for h in range(H)], axis=1)
        ctx_row = jnp.broadcast_to(ctx_row, (8, H * D)).astype(BF16)

        attn = jnp.zeros((8, M), F32)
        for g in range(NG):
            issue_gu(g)
            wait_filled(wo_v.at[pl.ds(g * 8, 8)], S_O + g)
            wo_g = wo_v[g * 8:(g + 1) * 8].reshape(8 * D, M)
            attn = attn + jnp.dot(ctx_row[:, g * 8 * D:(g + 1) * 8 * D], wo_g,
                                  preferred_element_type=F32)
        x1 = x0 + ga * attn
        h1 = (_layernorm(x1) * (1.0 + cb) + sb).astype(BF16)

        gate = jnp.zeros((8, Df), F32)
        up = jnp.zeros((8, Df), F32)
        for g in range(NG):
            for i in wd_plan[g]:
                issue_wd(i)
            wait_filled(wgu_v.at[g], S_GU + g)
            hk = h1[:, g * 128:(g + 1) * 128]
            gate = gate + jnp.dot(hk, wgu_v[g, 0], preferred_element_type=F32)
            up = up + jnp.dot(hk, wgu_v[g, 1], preferred_element_type=F32)
        hid = (_gelu_tanh(gate) * up).astype(BF16)

        f0 = Df - wv_rows
        hm = jnp.broadcast_to(hid[0:1, f0:].astype(F32), (128, wv_rows)).T
        y = jnp.zeros((8, M), F32)
        for i in range(n_mxu):
            o, n = wd_offs[i], wd_chunks[i]
            wait_filled(wd_v.at[pl.ds(o, n), :], S_D + i)
            y = y + jnp.dot(hid[:, o:o + n], wd_v[o:o + n, :], preferred_element_type=F32)
        row = lax.broadcasted_iota(jnp.int32, (8, M), 0)
        acc = jnp.where(row == 0, y, 0.0)
        for i in range(n_mxu, n_wd):
            o, n = wd_offs[i], wd_chunks[i]
            wait_filled(wd_v.at[pl.ds(o, n), :], S_D + i)
            for r in range(o, o + n, 16):
                wt = wd_v[r:r + 16, :].astype(F32)
                for t in range(2):
                    mul = hm[r - f0 + 8 * t:r - f0 + 8 * t + 8, :]
                    acc = acc + wt[8 * t:8 * t + 8] * jnp.concatenate([mul] * (M // 128), axis=1)
        out = x1[0:1] + gb[0:1] * jnp.sum(acc, axis=0, keepdims=True)
        o_ref[0] = out.astype(o_ref.dtype)

    any_spec = pl.BlockSpec(memory_space=pl.ANY)
    return pl.pallas_call(
        kernel,
        out_shape=jax.ShapeDtypeStruct(A_x.shape, A_x.dtype),
        in_specs=[any_spec] * 11,
        out_specs=pl.BlockSpec(memory_space=pltpu.VMEM),
        scratch_shapes=[
            pltpu.VMEM(A_x.shape, A_x.dtype),
            pltpu.VMEM(c.shape, c.dtype),
            pltpu.VMEM(w_mod.shape, w_mod.dtype),
            pltpu.VMEM(A_w_q.shape, A_w_q.dtype),
            pltpu.VMEM(A_w_uk.shape, A_w_uk.dtype),
            pltpu.VMEM((Sk, Dc), A_c_kv.dtype),
            pltpu.VMEM(A_w_uv.shape, A_w_uv.dtype),
            pltpu.VMEM(A_w_o.shape, A_w_o.dtype),
            pltpu.VMEM((NG, 2, M // NG, Df), B_w_gate.dtype),
            pltpu.VMEM(B_w_down.shape, B_w_down.dtype),
            pltpu.VMEM((M, 128), F32),
            pltpu.VMEM((NG, H, 128), F32),
            pltpu.VMEM((H, D), F32),
        ],
        compiler_params=pltpu.CompilerParams(vmem_limit_bytes=100 * 1024 * 1024),
    )(A_x, A_c_kv, A_w_q, A_w_uk, A_w_uv, A_w_o, B_w_gate, B_w_up, B_w_down, c, w_mod)
```

```python
import jax
import jax.numpy as jnp
from jax import lax
import jax.experimental.pallas as pl
import jax.experimental.pallas.tpu as pltpu

F32 = jnp.float32
BF16 = jnp.bfloat16
_NT = (((1,), (1,)), ((), ()))


def _layernorm(x, eps=1e-5):
    m = jnp.mean(x, axis=-1, keepdims=True)
    d = x - m
    v = jnp.mean(d * d, axis=-1, keepdims=True)
    return d * lax.rsqrt(v + eps)


def _gelu_tanh(x):
    c0 = 0.7978845608028654
    return 0.5 * x * (1.0 + jnp.tanh(c0 * (x + 0.044715 * (x * x * x))))


@jax.jit
def pallas_adaLN_cond__compressed_kv_cla__glu_gated_geglu__decode_kernel(
    A_x: jax.Array,
    A_c_kv: jax.Array,
    A_w_q: jax.Array,
    A_w_uk: jax.Array,
    A_w_uv: jax.Array,
    A_w_o: jax.Array,
    B_x: jax.Array,
    B_w_gate: jax.Array,
    B_w_up: jax.Array,
    B_w_down: jax.Array,
    c: jax.Array,
    w_mod: jax.Array,
):
    del B_x
    _, _, M = A_x.shape
    _, Sk, Dc = A_c_kv.shape
    _, H, D = A_w_q.shape
    Df = B_w_gate.shape[1]
    assert A_x.shape == (1, 1, 512) and A_c_kv.shape[0] == 1 and Dc == 512
    assert (H, D) == (32, 128) and Df == 1792 and w_mod.shape == (M, 6 * M)

    BK = 1024
    NG = 4
    LOOK = NG
    n_kv = Sk // BK
    assert Sk % BK == 0 and n_kv >= LOOK
    KV_S = 8
    KV_R = 32
    KV_PAT = (0, 1)
    KV_UNROLL = 1
    KV_SPLIT = 0
    kv_steps = BK // (KV_S * KV_R)
    kv_nstep = n_kv * kv_steps
    assert kv_steps * KV_S * KV_R == BK
    W3_S = 8
    W3_PAT = (0, 1)
    W3_R = 4
    WO_S = 8
    WO_PAT = (0, 1)
    MOD_S = 4
    MOD_PAT = (0, 1)
    GU_PAT = (0, 1)
    GU_NC = 2
    WD_R = 32
    w3_reg = 512 // W3_S
    w3_per = w3_reg // NG
    w3_steps = w3_per // W3_R
    assert w3_steps * W3_R * W3_S * NG == 512 and 128 % w3_reg == 0

    def w3_row(g, k, j):
        return j * w3_reg + g * w3_per + k * W3_R

    wo_per = 32 // WO_S // NG
    WD_MXU = [512, 512, 256, 256]
    WD_VPU = [128, 64, 32, 16, 16]
    WD_PAT = [(0, 1), (0, 1), (1,), (1,)]
    wv_rows = sum(WD_VPU)
    assert sum(WD_MXU) + wv_rows == Df and wv_rows % 128 == 0
    assert all(n % 128 == 0 for n in WD_MXU) and all(n % 16 == 0 for n in WD_VPU)
    wd_chunks = list(WD_MXU) + list(WD_VPU)
    wd_offs = [sum(wd_chunks[:i]) for i in range(len(wd_chunks))]
    n_mxu, n_wd = len(WD_MXU), len(wd_chunks)

    S_X, S_C, S_MOD = 0, 1, 2
    S_Q = 3
    S_UK = S_Q + NG
    S_KV = S_UK + NG
    S_UV = S_KV + n_kv
    S_O = S_UV + NG
    S_GU = S_O + NG
    S_D = S_GU + NG
    n_sem = S_D + n_wd
    scale = float(D) ** -0.5

    def kernel(*refs):
        pl.run_scoped(lambda sems: body(*refs, sems), pltpu.SemaphoreType.DMA((n_sem,)))

    def body(x_hbm, ckv_hbm, wq_hbm, wuk_hbm, wuv_hbm, wo_hbm, wg_hbm, wu_hbm, wd_hbm,
             c_hbm, wmod_hbm, o_ref,
             x_v, c_v, wmod_v, wq_v, wuk_v, ckv_v, wuv_v, wo_v, wgu_v, wd_v,
             hb_v, qa_v, ctx_v, sems):

        def start(src, dst, s, prio):
            pltpu.make_async_copy(src, dst, sems.at[s]).start(priority=prio)

        def wait_filled(buf, s):
            pltpu.make_async_copy(buf, buf, sems.at[s]).wait()

        def loop(n, step):
            lax.fori_loop(0, n, lambda k, _: step(k) or 0, 0)

        def issue_mod():
            bands = 32 // MOD_S

            def step(band):
                for third in range(3):
                    for j in range(MOD_S):
                        rows = pl.ds(pl.multiple_of((j * bands + band) * 16, 16), 16)
                        cols = pl.ds(third * 1024, 1024)
                        start(wmod_hbm.at[rows, cols], wmod_v.at[rows, cols], S_MOD,
                              MOD_PAT[j % len(MOD_PAT)])
            loop(bands, step)

        def issue_w3(hbm, vm, s0, g):
            def step(k):
                for j in range(W3_S):
                    dst = g * 128 + (k * W3_S + j) * W3_R
                    start(hbm.at[pl.ds(w3_row(g, k, j), W3_R)], vm.at[pl.ds(dst, W3_R)], s0 + g,
                          W3_PAT[j % len(W3_PAT)])
            loop(w3_steps, step)

        def wait_w3(vm, s0, g):
            wait_filled(vm.at[pl.ds(g * 128, 128)], s0 + g)

        def issue_kv(b, t0=0, t1=kv_steps):
            def step(t):
                k = b * kv_steps + t
                for j in range(KV_S):
                    src = (j * kv_nstep + k) * KV_R
                    dst = b * BK + (t * KV_S + j) * KV_R
                    start(ckv_hbm.at[0, pl.ds(pl.multiple_of(src, KV_R), KV_R), :],
                          ckv_v.at[pl.ds(pl.multiple_of(dst, KV_R), KV_R), :], S_KV + b,
                          KV_PAT[j % len(KV_PAT)])
            lax.fori_loop(t0, t1, lambda t, _: step(t) or 0, 0, unroll=KV_UNROLL)

        def issue_wo(g):
            def step(part):
                rows = pl.ds(pl.multiple_of(part * 32, 32), 32)
                for hh in range(wo_per):
                    for j in range(WO_S):
                        head = j * (32 // WO_S) + g * wo_per + hh
                        start(wo_hbm.at[head, rows, :], wo_v.at[g * 8 + hh * WO_S + j, rows, :],
                              S_O + g, WO_PAT[j % len(WO_PAT)])
            loop(4, step)

        def issue_gu(g):
            def step(k):
                rows = pl.ds(pl.multiple_of(g * 128 + k * 16, 16), 16)
                drows = pl.ds(pl.multiple_of(k * 16, 16), 16)
                for cp in range(GU_NC):
                    cols = pl.ds(cp * (Df // GU_NC), Df // GU_NC)
                    start(wg_hbm.at[rows, cols], wgu_v.at[g, 0, drows, cols], S_GU + g,
                          GU_PAT[(2 * cp) % len(GU_PAT)])
                    start(wu_hbm.at[rows, cols], wgu_v.at[g, 1, drows, cols], S_GU + g,
                          GU_PAT[(2 * cp + 1) % len(GU_PAT)])
            loop(8, step)

        def issue_wd(i):
            o, n = wd_offs[i], wd_chunks[i]
            pat = WD_PAT[i] if i < n_mxu else (1,)
            piece = min(n, WD_R)
            npc = n // piece
            if npc <= 2 * len(pat):
                for k in range(npc):
                    rows = pl.ds(o + k * piece, piece)
                    start(wd_hbm.at[rows, :], wd_v.at[rows, :], S_D + i, pat[k % len(pat)])
                return

            def step(k):
                for j, prio in enumerate(pat):
                    rows = pl.ds(pl.multiple_of(o + (k * len(pat) + j) * piece, piece), piece)
                    start(wd_hbm.at[rows, :], wd_v.at[rows, :], S_D + i, prio)
            loop(npc // len(pat), step)

        wd_plan = [[0], [1], [2], list(range(3, n_wd))] if n_mxu >= 4 else [list(range(n_wd)), [], [], []]

        start(x_hbm, x_v, S_X, 0)
        start(c_hbm, c_v, S_C, 0)
        issue_mod()
        for g in range(LOOK):
            issue_w3(wq_hbm, wq_v, S_Q, g)

        wait_filled(c_v, S_C)
        wait_filled(x_v, S_X)
        cvec = jnp.broadcast_to(c_v[...].astype(F32), (8, M))
        sc = (cvec * jax.nn.sigmoid(cvec)).astype(BF16)
        x0 = jnp.broadcast_to(x_v[0].astype(F32), (8, M))
        ln0 = _layernorm(x0)
        wait_filled(wmod_v, S_MOD)
        mod = jnp.dot(sc, wmod_v[...], preferred_element_type=F32)
        sa, ca, ga, sb, cb, gb = (mod[:, i * M:(i + 1) * M] for i in range(6))
        h0 = ln0 * (1.0 + ca) + sa
        hb_v[...] = jnp.broadcast_to(h0[0:1, :], (128, M)).T

        def q_group(g, acc):
            issue_w3(wuk_hbm, wuk_v, S_UK, g)
            wait_w3(wq_v, S_Q, g)

            def q_part(k, acc):
                for j in range(W3_S):
                    for t in range(W3_R):
                        pos = g * 128 + (k * W3_S + j) * W3_R + t
                        acc = acc + hb_v[pl.ds(w3_row(g, k, j) + t, 1), :] * wq_v[pos].astype(F32)
                return acc

            return lax.fori_loop(0, w3_steps, q_part, acc)

        q = lax.fori_loop(0, NG, q_group, jnp.zeros((H, D), F32)) * scale

        lane = lax.broadcasted_iota(jnp.int32, (H, 128), 1)

        def qa_group(g, accs):
            issue_kv(g)
            wait_w3(wuk_v, S_UK, g)
            lane_rel = lane - g * w3_per
            accs = list(accs)
            for k in range(w3_steps):
                for j in range(W3_S):
                    for t in range(W3_R):
                        pos = g * 128 + (k * W3_S + j) * W3_R + t
                        blk, ln = divmod(w3_row(0, k, j) + t, 128)
                        col = jnp.sum(q * wuk_v[pos].astype(F32), axis=1, keepdims=True)
                        accs[blk] = jnp.where(lane_rel == ln, col, accs[blk])
            return tuple(accs)

        accs = lax.fori_loop(0, NG, qa_group, tuple(jnp.zeros((H, 128), F32) for _ in range(NG)))
        qa = jnp.concatenate(accs, axis=1).astype(BF16)

        def kv_group(b, carry):
            @pl.when(b + LOOK < n_kv)
            def _():
                issue_kv(b + LOOK, 0, kv_steps - KV_SPLIT)

            @pl.when(b + LOOK >= n_kv)
            def _():
                issue_w3(wuv_hbm, wuv_v, S_UV, b + LOOK - n_kv)

            rows = pl.ds(pl.multiple_of(b * BK, BK), BK)
            wait_filled(ckv_v.at[rows, :], S_KV + b)
            m, l, acc = carry
            kv = ckv_v[rows, :]
            s = lax.dot_general(qa, kv, _NT, preferred_element_type=F32)
            mn = jnp.maximum(m, jnp.max(s, axis=1, keepdims=True))
            a = jnp.exp(m - mn)
            p = jnp.exp(s - mn)
            l = a * l + jnp.sum(p, axis=1, keepdims=True)
            if KV_SPLIT:
                @pl.when(b + LOOK < n_kv)
                def _():
                    issue_kv(b + LOOK, kv_steps - KV_SPLIT, kv_steps)
                kv = ckv_v[rows, :]
            acc = a * acc + jnp.dot(p.astype(BF16), kv, preferred_element_type=F32)
            return mn, l, acc

        init = (jnp.full((H, 1), -jnp.inf, F32), jnp.zeros((H, 1), F32), jnp.zeros((H, Dc), F32))
        _, l_fin, acc_fin = lax.fori_loop(0, n_kv, kv_group, init)
        ctxc = acc_fin / l_fin
        for i in range(NG):
            qa_v[i] = ctxc[:, i * 128:(i + 1) * 128]

        def ctx_group(g, acc):
            issue_wo(g)
            wait_w3(wuv_v, S_UV, g)
            shift = (128 - g * w3_per) % 128
            blks = [pltpu.roll(qa_v[i], shift, 1) for i in range(NG)]
            for k in range(w3_steps):
                for j in range(W3_S):
                    for t in range(W3_R):
                        pos = g * 128 + (k * W3_S + j) * W3_R + t
                        blk, ln = divmod(w3_row(0, k, j) + t, 128)
                        acc = acc + blks[blk][:, ln:ln + 1] * wuv_v[pos].astype(F32)
            return acc

        ctx_v[...] = lax.fori_loop(0, NG, ctx_group, jnp.zeros((H, D), F32))
        heads = [j * (32 // WO_S) + g * wo_per + hh
                 for g in range(NG) for hh in range(wo_per) for j in range(WO_S)]
        ctx_row = jnp.concatenate([ctx_v[h:h + 1, :] for h in heads], axis=1)
        ctx_row = jnp.broadcast_to(ctx_row, (8, H * D)).astype(BF16)

        attn = jnp.zeros((8, M), F32)
        for g in range(NG):
            issue_gu(g)
            wait_filled(wo_v.at[pl.ds(g * 8, 8)], S_O + g)
            wo_g = wo_v[g * 8:(g + 1) * 8].reshape(8 * D, M)
            attn = attn + jnp.dot(ctx_row[:, g * 8 * D:(g + 1) * 8 * D], wo_g,
                                  preferred_element_type=F32)
        x1 = x0 + ga * attn
        h1 = (_layernorm(x1) * (1.0 + cb) + sb).astype(BF16)

        gate = jnp.zeros((8, Df), F32)
        up = jnp.zeros((8, Df), F32)
        for g in range(NG):
            for i in wd_plan[g]:
                issue_wd(i)
            wait_filled(wgu_v.at[g], S_GU + g)
            hk = h1[:, g * 128:(g + 1) * 128]
            gate = gate + jnp.dot(hk, wgu_v[g, 0], preferred_element_type=F32)
            up = up + jnp.dot(hk, wgu_v[g, 1], preferred_element_type=F32)
        hid = (_gelu_tanh(gate) * up).astype(BF16)

        f0 = Df - wv_rows
        hm = jnp.broadcast_to(hid[0:1, f0:].astype(F32), (128, wv_rows)).T
        y = jnp.zeros((8, M), F32)
        for i in range(n_mxu):
            o, n = wd_offs[i], wd_chunks[i]
            wait_filled(wd_v.at[pl.ds(o, n), :], S_D + i)
            y = y + jnp.dot(hid[:, o:o + n], wd_v[o:o + n, :], preferred_element_type=F32)
        row = lax.broadcasted_iota(jnp.int32, (8, M), 0)
        acc = jnp.where(row == 0, y, 0.0)
        for i in range(n_mxu, n_wd):
            o, n = wd_offs[i], wd_chunks[i]
            wait_filled(wd_v.at[pl.ds(o, n), :], S_D + i)
            for r in range(o, o + n, 16):
                wt = wd_v[r:r + 16, :].astype(F32)
                for t in range(2):
                    mul = hm[r - f0 + 8 * t:r - f0 + 8 * t + 8, :]
                    acc = acc + wt[8 * t:8 * t + 8] * jnp.concatenate([mul] * (M // 128), axis=1)
        out = x1[0:1] + gb[0:1] * jnp.sum(acc, axis=0, keepdims=True)
        o_ref[0] = out.astype(o_ref.dtype)

    any_spec = pl.BlockSpec(memory_space=pl.ANY)
    return pl.pallas_call(
        kernel,
        out_shape=jax.ShapeDtypeStruct(A_x.shape, A_x.dtype),
        in_specs=[any_spec] * 11,
        out_specs=pl.BlockSpec(memory_space=pltpu.VMEM),
        scratch_shapes=[
            pltpu.VMEM(A_x.shape, A_x.dtype),
            pltpu.VMEM(c.shape, c.dtype),
            pltpu.VMEM(w_mod.shape, w_mod.dtype),
            pltpu.VMEM(A_w_q.shape, A_w_q.dtype),
            pltpu.VMEM(A_w_uk.shape, A_w_uk.dtype),
            pltpu.VMEM((Sk, Dc), A_c_kv.dtype),
            pltpu.VMEM(A_w_uv.shape, A_w_uv.dtype),
            pltpu.VMEM(A_w_o.shape, A_w_o.dtype),
            pltpu.VMEM((NG, 2, M // NG, Df), B_w_gate.dtype),
            pltpu.VMEM(B_w_down.shape, B_w_down.dtype),
            pltpu.VMEM((M, 128), F32),
            pltpu.VMEM((NG, H, 128), F32),
            pltpu.VMEM((H, D), F32),
        ],
        compiler_params=pltpu.CompilerParams(vmem_limit_bytes=100 * 1024 * 1024),
    )(A_x, A_c_kv, A_w_q, A_w_uk, A_w_uv, A_w_o, B_w_gate, B_w_up, B_w_down, c, w_mod)
```

```python
import jax
import jax.numpy as jnp
from jax import lax
import jax.experimental.pallas as pl
import jax.experimental.pallas.tpu as pltpu

F32 = jnp.float32
BF16 = jnp.bfloat16
_NT = (((1,), (1,)), ((), ()))


def _layernorm(x, eps=1e-5):
    m = jnp.mean(x, axis=-1, keepdims=True)
    d = x - m
    v = jnp.mean(d * d, axis=-1, keepdims=True)
    return d * lax.rsqrt(v + eps)


def _gelu_tanh(x):
    c0 = 0.7978845608028654
    return 0.5 * x * (1.0 + jnp.tanh(c0 * (x + 0.044715 * (x * x * x))))


@jax.jit
def pallas_adaLN_cond__compressed_kv_cla__glu_gated_geglu__decode_kernel(
    A_x: jax.Array,
    A_c_kv: jax.Array,
    A_w_q: jax.Array,
    A_w_uk: jax.Array,
    A_w_uv: jax.Array,
    A_w_o: jax.Array,
    B_x: jax.Array,
    B_w_gate: jax.Array,
    B_w_up: jax.Array,
    B_w_down: jax.Array,
    c: jax.Array,
    w_mod: jax.Array,
):
    del B_x
    _, _, M = A_x.shape
    _, Sk, Dc = A_c_kv.shape
    _, H, D = A_w_q.shape
    Df = B_w_gate.shape[1]
    assert A_x.shape == (1, 1, 512) and A_c_kv.shape[0] == 1 and Dc == 512
    assert (H, D) == (32, 128) and Df == 1792 and w_mod.shape == (M, 6 * M)

    BK = 1024
    NG = 4
    LOOK = NG
    n_kv = Sk // BK
    assert Sk % BK == 0 and n_kv >= LOOK
    KV_S = 8
    KV_R = 32
    KV_PAT = (0, 1)
    KV_UNROLL = 1
    KV_SPLIT = 0
    kv_steps = BK // (KV_S * KV_R)
    kv_nstep = n_kv * kv_steps
    assert kv_steps * KV_S * KV_R == BK
    W3_S = 8
    W3_PAT = (1, 1, 1, 0)
    W3_R = 4
    WO_S = 8
    WO_PAT = (0, 1, 1, 1)
    MOD_S = 4
    MOD_PAT = (0, 1, 1, 1)
    GU_PAT = (0, 1, 1, 1)
    GU_NC = 2
    WD_R = 32
    w3_reg = 512 // W3_S
    w3_per = w3_reg // NG
    w3_steps = w3_per // W3_R
    assert w3_steps * W3_R * W3_S * NG == 512 and 128 % w3_reg == 0

    def w3_row(g, k, j):
        return j * w3_reg + g * w3_per + k * W3_R

    wo_per = 32 // WO_S // NG
    WD_MXU = [512, 512, 256, 256]
    WD_VPU = [128, 64, 32, 16, 16]
    WD_PAT = [(0, 1), (0, 1), (1,), (1,)]
    wv_rows = sum(WD_VPU)
    assert sum(WD_MXU) + wv_rows == Df and wv_rows % 128 == 0
    assert all(n % 128 == 0 for n in WD_MXU) and all(n % 16 == 0 for n in WD_VPU)
    wd_chunks = list(WD_MXU) + list(WD_VPU)
    wd_offs = [sum(wd_chunks[:i]) for i in range(len(wd_chunks))]
    n_mxu, n_wd = len(WD_MXU), len(wd_chunks)

    S_X, S_C, S_MOD = 0, 1, 2
    S_Q = 3
    S_UK = S_Q + NG
    S_KV = S_UK + NG
    S_UV = S_KV + n_kv
    S_O = S_UV + NG
    S_GU = S_O + NG
    S_D = S_GU + NG
    n_sem = S_D + n_wd
    scale = float(D) ** -0.5

    def kernel(*refs):
        pl.run_scoped(lambda sems: body(*refs, sems), pltpu.SemaphoreType.DMA((n_sem,)))

    def body(x_hbm, ckv_hbm, wq_hbm, wuk_hbm, wuv_hbm, wo_hbm, wg_hbm, wu_hbm, wd_hbm,
             c_hbm, wmod_hbm, o_ref,
             x_v, c_v, wmod_v, wq_v, wuk_v, ckv_v, wuv_v, wo_v, wgu_v, wd_v,
             hb_v, qa_v, ctx_v, sems):

        def start(src, dst, s, prio):
            pltpu.make_async_copy(src, dst, sems.at[s]).start(priority=prio)

        def wait_filled(buf, s):
            pltpu.make_async_copy(buf, buf, sems.at[s]).wait()

        def loop(n, step):
            lax.fori_loop(0, n, lambda k, _: step(k) or 0, 0)

        def issue_mod():
            bands = 32 // MOD_S

            def step(band):
                for third in range(3):
                    for j in range(MOD_S):
                        rows = pl.ds(pl.multiple_of((j * bands + band) * 16, 16), 16)
                        cols = pl.ds(third * 1024, 1024)
                        start(wmod_hbm.at[rows, cols], wmod_v.at[rows, cols], S_MOD,
                              MOD_PAT[j % len(MOD_PAT)])
            loop(bands, step)

        def issue_w3(hbm, vm, s0, g):
            def step(k):
                for j in range(W3_S):
                    dst = g * 128 + (k * W3_S + j) * W3_R
                    start(hbm.at[pl.ds(w3_row(g, k, j), W3_R)], vm.at[pl.ds(dst, W3_R)], s0 + g,
                          W3_PAT[j % len(W3_PAT)])
            loop(w3_steps, step)

        def wait_w3(vm, s0, g):
            wait_filled(vm.at[pl.ds(g * 128, 128)], s0 + g)

        def issue_kv(b, t0=0, t1=kv_steps):
            def step(t):
                k = b * kv_steps + t
                for j in range(KV_S):
                    src = (j * kv_nstep + k) * KV_R
                    dst = b * BK + (t * KV_S + j) * KV_R
                    start(ckv_hbm.at[0, pl.ds(pl.multiple_of(src, KV_R), KV_R), :],
                          ckv_v.at[pl.ds(pl.multiple_of(dst, KV_R), KV_R), :], S_KV + b,
                          KV_PAT[j % len(KV_PAT)])
            lax.fori_loop(t0, t1, lambda t, _: step(t) or 0, 0, unroll=KV_UNROLL)

        def issue_wo(g):
            def step(part):
                rows = pl.ds(pl.multiple_of(part * 32, 32), 32)
                for hh in range(wo_per):
                    for j in range(WO_S):
                        head = j * (32 // WO_S) + g * wo_per + hh
                        start(wo_hbm.at[head, rows, :], wo_v.at[g * 8 + hh * WO_S + j, rows, :],
                              S_O + g, WO_PAT[j % len(WO_PAT)])
            loop(4, step)

        def issue_gu(g):
            def step(k):
                rows = pl.ds(pl.multiple_of(g * 128 + k * 16, 16), 16)
                drows = pl.ds(pl.multiple_of(k * 16, 16), 16)
                for cp in range(GU_NC):
                    cols = pl.ds(cp * (Df // GU_NC), Df // GU_NC)
                    start(wg_hbm.at[rows, cols], wgu_v.at[g, 0, drows, cols], S_GU + g,
                          GU_PAT[(2 * cp) % len(GU_PAT)])
                    start(wu_hbm.at[rows, cols], wgu_v.at[g, 1, drows, cols], S_GU + g,
                          GU_PAT[(2 * cp + 1) % len(GU_PAT)])
            loop(8, step)

        def issue_wd(i):
            o, n = wd_offs[i], wd_chunks[i]
            pat = WD_PAT[i] if i < n_mxu else (1,)
            piece = min(n, WD_R)
            npc = n // piece
            if npc <= 2 * len(pat):
                for k in range(npc):
                    rows = pl.ds(o + k * piece, piece)
                    start(wd_hbm.at[rows, :], wd_v.at[rows, :], S_D + i, pat[k % len(pat)])
                return

            def step(k):
                for j, prio in enumerate(pat):
                    rows = pl.ds(pl.multiple_of(o + (k * len(pat) + j) * piece, piece), piece)
                    start(wd_hbm.at[rows, :], wd_v.at[rows, :], S_D + i, prio)
            loop(npc // len(pat), step)

        wd_plan = [[0], [1], [2], list(range(3, n_wd))] if n_mxu >= 4 else [list(range(n_wd)), [], [], []]

        start(x_hbm, x_v, S_X, 0)
        start(c_hbm, c_v, S_C, 0)
        issue_mod()
        for g in range(LOOK):
            issue_w3(wq_hbm, wq_v, S_Q, g)

        wait_filled(c_v, S_C)
        wait_filled(x_v, S_X)
        cvec = jnp.broadcast_to(c_v[...].astype(F32), (8, M))
        sc = (cvec * jax.nn.sigmoid(cvec)).astype(BF16)
        x0 = jnp.broadcast_to(x_v[0].astype(F32), (8, M))
        ln0 = _layernorm(x0)
        wait_filled(wmod_v, S_MOD)
        mod = jnp.dot(sc, wmod_v[...], preferred_element_type=F32)
        sa, ca, ga, sb, cb, gb = (mod[:, i * M:(i + 1) * M] for i in range(6))
        h0 = ln0 * (1.0 + ca) + sa
        hb_v[...] = jnp.broadcast_to(h0[0:1, :], (128, M)).T

        def q_group(g, acc):
            issue_w3(wuk_hbm, wuk_v, S_UK, g)
            wait_w3(wq_v, S_Q, g)

            def q_part(k, acc):
                for j in range(W3_S):
                    for t in range(W3_R):
                        pos = g * 128 + (k * W3_S + j) * W3_R + t
                        acc = acc + hb_v[pl.ds(w3_row(g, k, j) + t, 1), :] * wq_v[pos].astype(F32)
                return acc

            return lax.fori_loop(0, w3_steps, q_part, acc)

        q = lax.fori_loop(0, NG, q_group, jnp.zeros((H, D), F32)) * scale

        lane = lax.broadcasted_iota(jnp.int32, (H, 128), 1)

        def qa_group(g, accs):
            issue_kv(g)
            wait_w3(wuk_v, S_UK, g)
            lane_rel = lane - g * w3_per
            accs = list(accs)
            for k in range(w3_steps):
                for j in range(W3_S):
                    for t in range(W3_R):
                        pos = g * 128 + (k * W3_S + j) * W3_R + t
                        blk, ln = divmod(w3_row(0, k, j) + t, 128)
                        col = jnp.sum(q * wuk_v[pos].astype(F32), axis=1, keepdims=True)
                        accs[blk] = jnp.where(lane_rel == ln, col, accs[blk])
            return tuple(accs)

        accs = lax.fori_loop(0, NG, qa_group, tuple(jnp.zeros((H, 128), F32) for _ in range(NG)))
        qa = jnp.concatenate(accs, axis=1).astype(BF16)

        def kv_group(b, carry):
            @pl.when(b + LOOK < n_kv)
            def _():
                issue_kv(b + LOOK, 0, kv_steps - KV_SPLIT)

            @pl.when(b + LOOK >= n_kv)
            def _():
                issue_w3(wuv_hbm, wuv_v, S_UV, b + LOOK - n_kv)

            rows = pl.ds(pl.multiple_of(b * BK, BK), BK)
            wait_filled(ckv_v.at[rows, :], S_KV + b)
            m, l, acc = carry
            kv = ckv_v[rows, :]
            s = lax.dot_general(qa, kv, _NT, preferred_element_type=F32)
            mn = jnp.maximum(m, jnp.max(s, axis=1, keepdims=True))
            a = jnp.exp(m - mn)
            p = jnp.exp(s - mn)
            l = a * l + jnp.sum(p, axis=1, keepdims=True)
            if KV_SPLIT:
                @pl.when(b + LOOK < n_kv)
                def _():
                    issue_kv(b + LOOK, kv_steps - KV_SPLIT, kv_steps)
                kv = ckv_v[rows, :]
            acc = a * acc + jnp.dot(p.astype(BF16), kv, preferred_element_type=F32)
            return mn, l, acc

        init = (jnp.full((H, 1), -jnp.inf, F32), jnp.zeros((H, 1), F32), jnp.zeros((H, Dc), F32))
        _, l_fin, acc_fin = lax.fori_loop(0, n_kv, kv_group, init)
        ctxc = acc_fin / l_fin
        for i in range(NG):
            qa_v[i] = ctxc[:, i * 128:(i + 1) * 128]

        def ctx_group(g, acc):
            issue_wo(g)
            wait_w3(wuv_v, S_UV, g)
            shift = (128 - g * w3_per) % 128
            blks = [pltpu.roll(qa_v[i], shift, 1) for i in range(NG)]
            for k in range(w3_steps):
                for j in range(W3_S):
                    for t in range(W3_R):
                        pos = g * 128 + (k * W3_S + j) * W3_R + t
                        blk, ln = divmod(w3_row(0, k, j) + t, 128)
                        acc = acc + blks[blk][:, ln:ln + 1] * wuv_v[pos].astype(F32)
            return acc

        ctx_v[...] = lax.fori_loop(0, NG, ctx_group, jnp.zeros((H, D), F32))
        heads = [j * (32 // WO_S) + g * wo_per + hh
                 for g in range(NG) for hh in range(wo_per) for j in range(WO_S)]
        ctx_row = jnp.concatenate([ctx_v[h:h + 1, :] for h in heads], axis=1)
        ctx_row = jnp.broadcast_to(ctx_row, (8, H * D)).astype(BF16)

        attn = jnp.zeros((8, M), F32)
        for g in range(NG):
            issue_gu(g)
            wait_filled(wo_v.at[pl.ds(g * 8, 8)], S_O + g)
            wo_g = wo_v[g * 8:(g + 1) * 8].reshape(8 * D, M)
            attn = attn + jnp.dot(ctx_row[:, g * 8 * D:(g + 1) * 8 * D], wo_g,
                                  preferred_element_type=F32)
        x1 = x0 + ga * attn
        h1 = (_layernorm(x1) * (1.0 + cb) + sb).astype(BF16)

        gate = jnp.zeros((8, Df), F32)
        up = jnp.zeros((8, Df), F32)
        for g in range(NG):
            for i in wd_plan[g]:
                issue_wd(i)
            wait_filled(wgu_v.at[g], S_GU + g)
            hk = h1[:, g * 128:(g + 1) * 128]
            gate = gate + jnp.dot(hk, wgu_v[g, 0], preferred_element_type=F32)
            up = up + jnp.dot(hk, wgu_v[g, 1], preferred_element_type=F32)
        hid = (_gelu_tanh(gate) * up).astype(BF16)

        f0 = Df - wv_rows
        hm = jnp.broadcast_to(hid[0:1, f0:].astype(F32), (128, wv_rows)).T
        y = jnp.zeros((8, M), F32)
        for i in range(n_mxu):
            o, n = wd_offs[i], wd_chunks[i]
            wait_filled(wd_v.at[pl.ds(o, n), :], S_D + i)
            y = y + jnp.dot(hid[:, o:o + n], wd_v[o:o + n, :], preferred_element_type=F32)
        row = lax.broadcasted_iota(jnp.int32, (8, M), 0)
        acc = jnp.where(row == 0, y, 0.0)
        for i in range(n_mxu, n_wd):
            o, n = wd_offs[i], wd_chunks[i]
            wait_filled(wd_v.at[pl.ds(o, n), :], S_D + i)
            for r in range(o, o + n, 16):
                wt = wd_v[r:r + 16, :].astype(F32)
                for t in range(2):
                    mul = hm[r - f0 + 8 * t:r - f0 + 8 * t + 8, :]
                    acc = acc + wt[8 * t:8 * t + 8] * jnp.concatenate([mul] * (M // 128), axis=1)
        out = x1[0:1] + gb[0:1] * jnp.sum(acc, axis=0, keepdims=True)
        o_ref[0] = out.astype(o_ref.dtype)

    any_spec = pl.BlockSpec(memory_space=pl.ANY)
    return pl.pallas_call(
        kernel,
        out_shape=jax.ShapeDtypeStruct(A_x.shape, A_x.dtype),
        in_specs=[any_spec] * 11,
        out_specs=pl.BlockSpec(memory_space=pltpu.VMEM),
        scratch_shapes=[
            pltpu.VMEM(A_x.shape, A_x.dtype),
            pltpu.VMEM(c.shape, c.dtype),
            pltpu.VMEM(w_mod.shape, w_mod.dtype),
            pltpu.VMEM(A_w_q.shape, A_w_q.dtype),
            pltpu.VMEM(A_w_uk.shape, A_w_uk.dtype),
            pltpu.VMEM((Sk, Dc), A_c_kv.dtype),
            pltpu.VMEM(A_w_uv.shape, A_w_uv.dtype),
            pltpu.VMEM(A_w_o.shape, A_w_o.dtype),
            pltpu.VMEM((NG, 2, M // NG, Df), B_w_gate.dtype),
            pltpu.VMEM(B_w_down.shape, B_w_down.dtype),
            pltpu.VMEM((M, 128), F32),
            pltpu.VMEM((NG, H, 128), F32),
            pltpu.VMEM((H, D), F32),
        ],
        compiler_params=pltpu.CompilerParams(vmem_limit_bytes=100 * 1024 * 1024),
    )(A_x, A_c_kv, A_w_q, A_w_uk, A_w_uv, A_w_o, B_w_gate, B_w_up, B_w_down, c, w_mod)
```

```python
import jax
import jax.numpy as jnp
from jax import lax
import jax.experimental.pallas as pl
import jax.experimental.pallas.tpu as pltpu

F32 = jnp.float32
BF16 = jnp.bfloat16
_NT = (((1,), (1,)), ((), ()))


def _layernorm(x, eps=1e-5):
    m = jnp.mean(x, axis=-1, keepdims=True)
    d = x - m
    v = jnp.mean(d * d, axis=-1, keepdims=True)
    return d * lax.rsqrt(v + eps)


def _gelu_tanh(x):
    c0 = 0.7978845608028654
    return 0.5 * x * (1.0 + jnp.tanh(c0 * (x + 0.044715 * (x * x * x))))


@jax.jit
def pallas_adaLN_cond__compressed_kv_cla__glu_gated_geglu__decode_kernel(
    A_x: jax.Array,
    A_c_kv: jax.Array,
    A_w_q: jax.Array,
    A_w_uk: jax.Array,
    A_w_uv: jax.Array,
    A_w_o: jax.Array,
    B_x: jax.Array,
    B_w_gate: jax.Array,
    B_w_up: jax.Array,
    B_w_down: jax.Array,
    c: jax.Array,
    w_mod: jax.Array,
):
    del B_x
    _, _, M = A_x.shape
    _, Sk, Dc = A_c_kv.shape
    _, H, D = A_w_q.shape
    Df = B_w_gate.shape[1]
    assert A_x.shape == (1, 1, 512) and A_c_kv.shape[0] == 1 and Dc == 512
    assert (H, D) == (32, 128) and Df == 1792 and w_mod.shape == (M, 6 * M)

    BK = 1024
    NG = 4
    LOOK = NG
    n_kv = Sk // BK
    assert Sk % BK == 0 and n_kv >= LOOK
    KV_S = 8
    KV_R = 32
    KV_PAT = (0, 1)
    kv_steps = BK // (KV_S * KV_R)
    kv_nstep = n_kv * kv_steps
    assert kv_steps * KV_S * KV_R == BK
    W3_S = 8
    W3_R = 4
    W3_PAT = (1, 1, 1, 0)
    w3_reg = 512 // W3_S
    w3_per = w3_reg // NG
    w3_steps = w3_per // W3_R
    assert w3_steps * W3_R * W3_S * NG == 512 and 128 % w3_reg == 0

    def w3_row(g, k, j):
        return j * w3_reg + g * w3_per + k * W3_R

    WO_S = 8
    WO_PAT = (0, 1, 1, 1)
    wo_per = H // WO_S // NG
    MOD_S = 4
    MOD_PAT = (0, 1, 1, 1)
    GU_NC = 2
    GU_PAT = (0, 1, 1, 1)
    WD_MXU = [512, 512, 256, 256]
    WD_VPU = [128, 64, 32, 16, 16]
    WD_PAT = [(0, 1), (0, 1), (1,), (1,)]
    WD_R = 32
    wv_rows = sum(WD_VPU)
    assert sum(WD_MXU) + wv_rows == Df and wv_rows % 128 == 0
    assert all(n % 128 == 0 for n in WD_MXU) and all(n % 16 == 0 for n in WD_VPU)
    wd_chunks = list(WD_MXU) + list(WD_VPU)
    wd_offs = [sum(wd_chunks[:i]) for i in range(len(wd_chunks))]
    n_mxu, n_wd = len(WD_MXU), len(wd_chunks)

    S_X, S_C, S_MOD = 0, 1, 2
    S_Q = 3
    S_UK = S_Q + NG
    S_KV = S_UK + NG
    S_UV = S_KV + n_kv
    S_O = S_UV + NG
    S_GU = S_O + NG
    S_D = S_GU + NG
    n_sem = S_D + n_wd
    scale = float(D) ** -0.5

    def kernel(*refs):
        pl.run_scoped(lambda sems: body(*refs, sems), pltpu.SemaphoreType.DMA((n_sem,)))

    def body(x_hbm, ckv_hbm, wq_hbm, wuk_hbm, wuv_hbm, wo_hbm, wg_hbm, wu_hbm, wd_hbm,
             c_hbm, wmod_hbm, o_ref,
             x_v, c_v, wmod_v, wq_v, wuk_v, ckv_v, wuv_v, wo_v, wgu_v, wd_v,
             hb_v, qa_v, ctx_v, sems):

        def start(src, dst, s, prio):
            pltpu.make_async_copy(src, dst, sems.at[s]).start(priority=prio)

        def wait_filled(buf, s):
            pltpu.make_async_copy(buf, buf, sems.at[s]).wait()

        def loop(n, step):
            lax.fori_loop(0, n, lambda k, _: step(k) or 0, 0)

        def issue_mod():
            bands = 32 // MOD_S

            def step(band):
                for third in range(3):
                    for j in range(MOD_S):
                        rows = pl.ds(pl.multiple_of((j * bands + band) * 16, 16), 16)
                        cols = pl.ds(third * 1024, 1024)
                        start(wmod_hbm.at[rows, cols], wmod_v.at[rows, cols], S_MOD,
                              MOD_PAT[j % len(MOD_PAT)])
            loop(bands, step)

        def issue_w3(hbm, vm, s0, g):
            def step(k):
                for j in range(W3_S):
                    dst = g * 128 + (k * W3_S + j) * W3_R
                    start(hbm.at[pl.ds(w3_row(g, k, j), W3_R)], vm.at[pl.ds(dst, W3_R)], s0 + g,
                          W3_PAT[j % len(W3_PAT)])
            loop(w3_steps, step)

        def wait_w3(vm, s0, g):
            wait_filled(vm.at[pl.ds(g * 128, 128)], s0 + g)

        def issue_kv(b):
            def step(t):
                k = b * kv_steps + t
                for j in range(KV_S):
                    src = (j * kv_nstep + k) * KV_R
                    dst = b * BK + (t * KV_S + j) * KV_R
                    start(ckv_hbm.at[0, pl.ds(pl.multiple_of(src, KV_R), KV_R), :],
                          ckv_v.at[pl.ds(pl.multiple_of(dst, KV_R), KV_R), :], S_KV + b,
                          KV_PAT[j % len(KV_PAT)])
            loop(kv_steps, step)

        def issue_wo(g):
            def step(part):
                rows = pl.ds(pl.multiple_of(part * 32, 32), 32)
                for hh in range(wo_per):
                    for j in range(WO_S):
                        head = j * (H // WO_S) + g * wo_per + hh
                        start(wo_hbm.at[head, rows, :], wo_v.at[g * 8 + hh * WO_S + j, rows, :],
                              S_O + g, WO_PAT[j % len(WO_PAT)])
            loop(4, step)

        def issue_gu(g):
            def step(k):
                rows = pl.ds(pl.multiple_of(g * 128 + k * 16, 16), 16)
                drows = pl.ds(pl.multiple_of(k * 16, 16), 16)
                for cp in range(GU_NC):
                    cols = pl.ds(cp * (Df // GU_NC), Df // GU_NC)
                    start(wg_hbm.at[rows, cols], wgu_v.at[g, 0, drows, cols], S_GU + g,
                          GU_PAT[(2 * cp) % len(GU_PAT)])
                    start(wu_hbm.at[rows, cols], wgu_v.at[g, 1, drows, cols], S_GU + g,
                          GU_PAT[(2 * cp + 1) % len(GU_PAT)])
            loop(8, step)

        def issue_wd(i):
            o, n = wd_offs[i], wd_chunks[i]
            pat = WD_PAT[i] if i < n_mxu else (1,)
            piece = min(n, WD_R)
            npc = n // piece
            if npc <= 2 * len(pat):
                for k in range(npc):
                    rows = pl.ds(o + k * piece, piece)
                    start(wd_hbm.at[rows, :], wd_v.at[rows, :], S_D + i, pat[k % len(pat)])
                return

            def step(k):
                for j, prio in enumerate(pat):
                    rows = pl.ds(pl.multiple_of(o + (k * len(pat) + j) * piece, piece), piece)
                    start(wd_hbm.at[rows, :], wd_v.at[rows, :], S_D + i, prio)
            loop(npc // len(pat), step)

        wd_plan = [[0], [1], [2], list(range(3, n_wd))] if n_mxu >= 4 else [list(range(n_wd)), [], [], []]

        start(x_hbm, x_v, S_X, 0)
        start(c_hbm, c_v, S_C, 0)
        issue_mod()
        for g in range(LOOK):
            issue_w3(wq_hbm, wq_v, S_Q, g)

        wait_filled(c_v, S_C)
        wait_filled(x_v, S_X)
        cvec = jnp.broadcast_to(c_v[...].astype(F32), (8, M))
        sc = (cvec * jax.nn.sigmoid(cvec)).astype(BF16)
        x0 = jnp.broadcast_to(x_v[0].astype(F32), (8, M))
        ln0 = _layernorm(x0)
        wait_filled(wmod_v, S_MOD)
        mod = jnp.dot(sc, wmod_v[...], preferred_element_type=F32)
        sa, ca, ga, sb, cb, gb = (mod[:, i * M:(i + 1) * M] for i in range(6))
        h0 = ln0 * (1.0 + ca) + sa
        hb_v[...] = jnp.broadcast_to(h0[0:1, :], (128, M)).T

        def q_group(g, acc):
            issue_w3(wuk_hbm, wuk_v, S_UK, g)
            wait_w3(wq_v, S_Q, g)

            def q_part(k, acc):
                for j in range(W3_S):
                    for t in range(W3_R):
                        pos = g * 128 + (k * W3_S + j) * W3_R + t
                        acc = acc + hb_v[pl.ds(w3_row(g, k, j) + t, 1), :] * wq_v[pos].astype(F32)
                return acc

            return lax.fori_loop(0, w3_steps, q_part, acc)

        q = lax.fori_loop(0, NG, q_group, jnp.zeros((H, D), F32)) * scale

        lane = lax.broadcasted_iota(jnp.int32, (H, 128), 1)

        def qa_group(g, accs):
            issue_kv(g)
            wait_w3(wuk_v, S_UK, g)
            lane_rel = lane - g * w3_per
            accs = list(accs)
            for k in range(w3_steps):
                for j in range(W3_S):
                    for t in range(W3_R):
                        pos = g * 128 + (k * W3_S + j) * W3_R + t
                        blk, ln = divmod(w3_row(0, k, j) + t, 128)
                        col = jnp.sum(q * wuk_v[pos].astype(F32), axis=1, keepdims=True)
                        accs[blk] = jnp.where(lane_rel == ln, col, accs[blk])
            return tuple(accs)

        accs = lax.fori_loop(0, NG, qa_group, tuple(jnp.zeros((H, 128), F32) for _ in range(NG)))
        qa = jnp.concatenate(accs, axis=1).astype(BF16)

        def kv_group(b, carry):
            @pl.when(b + LOOK < n_kv)
            def _():
                issue_kv(b + LOOK)

            @pl.when(b + LOOK >= n_kv)
            def _():
                issue_w3(wuv_hbm, wuv_v, S_UV, b + LOOK - n_kv)

            rows = pl.ds(pl.multiple_of(b * BK, BK), BK)
            wait_filled(ckv_v.at[rows, :], S_KV + b)
            m, l, acc = carry
            kv = ckv_v[rows, :]
            s = lax.dot_general(qa, kv, _NT, preferred_element_type=F32)
            mn = jnp.maximum(m, jnp.max(s, axis=1, keepdims=True))
            a = jnp.exp(m - mn)
            p = jnp.exp(s - mn)
            l = a * l + jnp.sum(p, axis=1, keepdims=True)
            acc = a * acc + jnp.dot(p.astype(BF16), kv, preferred_element_type=F32)
            return mn, l, acc

        init = (jnp.full((H, 1), -jnp.inf, F32), jnp.zeros((H, 1), F32), jnp.zeros((H, Dc), F32))
        _, l_fin, acc_fin = lax.fori_loop(0, n_kv, kv_group, init)
        ctxc = acc_fin / l_fin
        for i in range(NG):
            qa_v[i] = ctxc[:, i * 128:(i + 1) * 128]

        def ctx_group(g, acc):
            issue_wo(g)
            wait_w3(wuv_v, S_UV, g)
            shift = (128 - g * w3_per) % 128
            blks = [pltpu.roll(qa_v[i], shift, 1) for i in range(NG)]
            for k in range(w3_steps):
                for j in range(W3_S):
                    for t in range(W3_R):
                        pos = g * 128 + (k * W3_S + j) * W3_R + t
                        blk, ln = divmod(w3_row(0, k, j) + t, 128)
                        acc = acc + blks[blk][:, ln:ln + 1] * wuv_v[pos].astype(F32)
            return acc

        ctx_v[...] = lax.fori_loop(0, NG, ctx_group, jnp.zeros((H, D), F32))
        heads = [j * (H // WO_S) + g * wo_per + hh
                 for g in range(NG) for hh in range(wo_per) for j in range(WO_S)]
        ctx_row = jnp.concatenate([ctx_v[h:h + 1, :] for h in heads], axis=1)
        ctx_row = jnp.broadcast_to(ctx_row, (8, H * D)).astype(BF16)

        attn = jnp.zeros((8, M), F32)
        for g in range(NG):
            issue_gu(g)
            wait_filled(wo_v.at[pl.ds(g * 8, 8)], S_O + g)
            wo_g = wo_v[g * 8:(g + 1) * 8].reshape(8 * D, M)
            attn = attn + jnp.dot(ctx_row[:, g * 8 * D:(g + 1) * 8 * D], wo_g,
                                  preferred_element_type=F32)
        x1 = x0 + ga * attn
        h1 = (_layernorm(x1) * (1.0 + cb) + sb).astype(BF16)

        gate = jnp.zeros((8, Df), F32)
        up = jnp.zeros((8, Df), F32)
        for g in range(NG):
            for i in wd_plan[g]:
                issue_wd(i)
            wait_filled(wgu_v.at[g], S_GU + g)
            hk = h1[:, g * 128:(g + 1) * 128]
            gate = gate + jnp.dot(hk, wgu_v[g, 0], preferred_element_type=F32)
            up = up + jnp.dot(hk, wgu_v[g, 1], preferred_element_type=F32)
        hid = (_gelu_tanh(gate) * up).astype(BF16)

        f0 = Df - wv_rows
        hm = jnp.broadcast_to(hid[0:1, f0:].astype(F32), (128, wv_rows)).T
        y = jnp.zeros((8, M), F32)
        for i in range(n_mxu):
            o, n = wd_offs[i], wd_chunks[i]
            wait_filled(wd_v.at[pl.ds(o, n), :], S_D + i)
            y = y + jnp.dot(hid[:, o:o + n], wd_v[o:o + n, :], preferred_element_type=F32)
        row = lax.broadcasted_iota(jnp.int32, (8, M), 0)
        acc = jnp.where(row == 0, y, 0.0)
        for i in range(n_mxu, n_wd):
            o, n = wd_offs[i], wd_chunks[i]
            wait_filled(wd_v.at[pl.ds(o, n), :], S_D + i)
            for r in range(o, o + n, 16):
                wt = wd_v[r:r + 16, :].astype(F32)
                for t in range(2):
                    mul = hm[r - f0 + 8 * t:r - f0 + 8 * t + 8, :]
                    acc = acc + wt[8 * t:8 * t + 8] * jnp.concatenate([mul] * (M // 128), axis=1)
        out = x1[0:1] + gb[0:1] * jnp.sum(acc, axis=0, keepdims=True)
        o_ref[0] = out.astype(o_ref.dtype)

    any_spec = pl.BlockSpec(memory_space=pl.ANY)
    return pl.pallas_call(
        kernel,
        out_shape=jax.ShapeDtypeStruct(A_x.shape, A_x.dtype),
        in_specs=[any_spec] * 11,
        out_specs=pl.BlockSpec(memory_space=pltpu.VMEM),
        scratch_shapes=[
            pltpu.VMEM(A_x.shape, A_x.dtype),
            pltpu.VMEM(c.shape, c.dtype),
            pltpu.VMEM(w_mod.shape, w_mod.dtype),
            pltpu.VMEM(A_w_q.shape, A_w_q.dtype),
            pltpu.VMEM(A_w_uk.shape, A_w_uk.dtype),
            pltpu.VMEM((Sk, Dc), A_c_kv.dtype),
            pltpu.VMEM(A_w_uv.shape, A_w_uv.dtype),
            pltpu.VMEM(A_w_o.shape, A_w_o.dtype),
            pltpu.VMEM((NG, 2, M // NG, Df), B_w_gate.dtype),
            pltpu.VMEM(B_w_down.shape, B_w_down.dtype),
            pltpu.VMEM((M, 128), F32),
            pltpu.VMEM((NG, H, 128), F32),
            pltpu.VMEM((H, D), F32),
        ],
        compiler_params=pltpu.CompilerParams(vmem_limit_bytes=100 * 1024 * 1024),
    )(A_x, A_c_kv, A_w_q, A_w_uk, A_w_uv, A_w_o, B_w_gate, B_w_up, B_w_down, c, w_mod)
```

```python
import jax
import jax.numpy as jnp
from jax import lax
import jax.experimental.pallas as pl
import jax.experimental.pallas.tpu as pltpu

F32 = jnp.float32
BF16 = jnp.bfloat16
_NT = (((1,), (1,)), ((), ()))


def _layernorm(x, eps=1e-5):
    m = jnp.mean(x, axis=-1, keepdims=True)
    d = x - m
    v = jnp.mean(d * d, axis=-1, keepdims=True)
    return d * lax.rsqrt(v + eps)


def _gelu_tanh(x):
    c0 = 0.7978845608028654
    return 0.5 * x * (1.0 + jnp.tanh(c0 * (x + 0.044715 * (x * x * x))))


@jax.jit
def pallas_adaLN_cond__compressed_kv_cla__glu_gated_geglu__decode_kernel(
    A_x: jax.Array,
    A_c_kv: jax.Array,
    A_w_q: jax.Array,
    A_w_uk: jax.Array,
    A_w_uv: jax.Array,
    A_w_o: jax.Array,
    B_x: jax.Array,
    B_w_gate: jax.Array,
    B_w_up: jax.Array,
    B_w_down: jax.Array,
    c: jax.Array,
    w_mod: jax.Array,
):
    del B_x
    _, _, M = A_x.shape
    _, Sk, Dc = A_c_kv.shape
    _, H, D = A_w_q.shape
    Df = B_w_gate.shape[1]
    assert A_x.shape == (1, 1, 512) and A_c_kv.shape[0] == 1 and Dc == 512
    assert (H, D) == (32, 128) and Df == 1792 and w_mod.shape == (M, 6 * M)

    BK = 1024
    NG = 4
    LOOK = NG
    n_kv = Sk // BK
    assert Sk % BK == 0 and n_kv >= LOOK
    KV_S = 16
    KV_R = 16
    KV_J = 2
    KV_PAT = (0, 1)
    kv_steps = BK // (KV_S * KV_R)
    kv_nstep = n_kv * kv_steps
    kv_ncp = KV_S // KV_J
    assert kv_steps * KV_S * KV_R == BK
    W3_S = 8
    W3_R = 4
    W3_J = 1
    W3_PAT = (1, 1, 1, 0)
    w3_reg = 512 // W3_S
    w3_per = w3_reg // NG
    w3_steps = w3_per // W3_R
    w3_ncp = W3_S // W3_J
    assert w3_steps * W3_R * W3_S * NG == 512 and 128 % w3_reg == 0
    w3_vshape = (NG * w3_steps * w3_ncp, W3_J, W3_R, H, D)

    def w3_at(vm, g, k, j, t):
        return vm[(g * w3_steps + k) * w3_ncp + j // W3_J, j % W3_J, t]

    def w3_row(g, k, j):
        return j * w3_reg + g * w3_per + k * W3_R

    WO_S = 8
    WO_PAT = (0, 1, 1, 1)
    WO_J = 1
    WO_R = 32
    wo_per = H // WO_S // NG
    MOD_S = 4
    MOD_PAT = (0, 1, 1, 1)
    GU_NC = 2
    GU_PAT = (0, 1, 1, 1)
    WD_MXU = [512, 512, 256, 256]
    WD_VPU = [128, 64, 32, 16, 16]
    WD_PAT = [(0, 1), (0, 1), (1,), (1,)]
    WD_R = 32
    wv_rows = sum(WD_VPU)
    assert sum(WD_MXU) + wv_rows == Df and wv_rows % 128 == 0
    assert all(n % 128 == 0 for n in WD_MXU) and all(n % 16 == 0 for n in WD_VPU)
    wd_chunks = list(WD_MXU) + list(WD_VPU)
    wd_offs = [sum(wd_chunks[:i]) for i in range(len(wd_chunks))]
    n_mxu, n_wd = len(WD_MXU), len(wd_chunks)

    S_X, S_C, S_MOD = 0, 1, 2
    S_Q = 3
    S_UK = S_Q + NG
    S_KV = S_UK + NG
    S_UV = S_KV + n_kv
    S_O = S_UV + NG
    S_GU = S_O + NG
    S_D = S_GU + NG
    n_sem = S_D + n_wd
    scale = float(D) ** -0.5

    def kernel(*refs):
        pl.run_scoped(lambda sems: body(*refs, sems), pltpu.SemaphoreType.DMA((n_sem,)))

    def body(x_hbm, ckv_hbm, wq_hbm, wuk_hbm, wuv_hbm, wo_hbm, wg_hbm, wu_hbm, wd_hbm,
             c_hbm, wmod_hbm, o_ref,
             x_v, c_v, wmod_v, wq_v, wuk_v, ckv_v, wuv_v, wo_v, wgu_v, wd_v,
             hb_v, qa_v, ctx_v, sems):

        def start(src, dst, s, prio):
            pltpu.make_async_copy(src, dst, sems.at[s]).start(priority=prio)

        def wait_filled(buf, s):
            pltpu.make_async_copy(buf, buf, sems.at[s]).wait()

        def loop(n, step):
            lax.fori_loop(0, n, lambda k, _: step(k) or 0, 0)

        def issue_mod():
            bands = 32 // MOD_S

            def step(band):
                for third in range(3):
                    for j in range(MOD_S):
                        rows = pl.ds(pl.multiple_of((j * bands + band) * 16, 16), 16)
                        cols = pl.ds(third * 1024, 1024)
                        start(wmod_hbm.at[rows, cols], wmod_v.at[rows, cols], S_MOD,
                              MOD_PAT[j % len(MOD_PAT)])
            loop(bands, step)

        def issue_w3(hbm, vm, s0, g):
            def step(k):
                for jj in range(w3_ncp):
                    start(hbm.at[pl.ds(jj * W3_J, W3_J), pl.ds(g * w3_per + k * W3_R, W3_R)],
                          vm.at[(g * w3_steps + k) * w3_ncp + jj], s0 + g,
                          W3_PAT[jj % len(W3_PAT)])
            loop(w3_steps, step)

        def wait_w3(vm, s0, g):
            wait_filled(vm.at[pl.ds(g * (w3_steps * w3_ncp), w3_steps * w3_ncp)], s0 + g)

        def issue_kv(b):
            def step(t):
                k = b * kv_steps + t
                rows = pl.ds(pl.multiple_of(k * KV_R, KV_R), KV_R)
                for jj in range(kv_ncp):
                    start(ckv_hbm.at[pl.ds(jj * KV_J, KV_J), rows, :],
                          ckv_v.at[k * kv_ncp + jj], S_KV + b, KV_PAT[jj % len(KV_PAT)])
            loop(kv_steps, step)

        def issue_wo(g):
            def step(part):
                rows = pl.ds(pl.multiple_of(part * WO_R, WO_R), WO_R)
                for hh in range(wo_per):
                    for jj in range(WO_S // WO_J):
                        regs = pl.ds(jj * WO_J, WO_J)
                        start(wo_hbm.at[regs, g * wo_per + hh, rows, :],
                              wo_v.at[g * wo_per + hh, regs, rows, :],
                              S_O + g, WO_PAT[jj % len(WO_PAT)])
            loop(D // WO_R, step)

        def issue_gu(g):
            def step(k):
                rows = pl.ds(pl.multiple_of(g * 128 + k * 16, 16), 16)
                drows = pl.ds(pl.multiple_of(k * 16, 16), 16)
                for cp in range(GU_NC):
                    cols = pl.ds(cp * (Df // GU_NC), Df // GU_NC)
                    start(wg_hbm.at[rows, cols], wgu_v.at[g, 0, drows, cols], S_GU + g,
                          GU_PAT[(2 * cp) % len(GU_PAT)])
                    start(wu_hbm.at[rows, cols], wgu_v.at[g, 1, drows, cols], S_GU + g,
                          GU_PAT[(2 * cp + 1) % len(GU_PAT)])
            loop(8, step)

        def issue_wd(i):
            o, n = wd_offs[i], wd_chunks[i]
            pat = WD_PAT[i] if i < n_mxu else (1,)
            piece = min(n, WD_R)
            npc = n // piece
            if npc <= 2 * len(pat):
                for k in range(npc):
                    rows = pl.ds(o + k * piece, piece)
                    start(wd_hbm.at[rows, :], wd_v.at[rows, :], S_D + i, pat[k % len(pat)])
                return

            def step(k):
                for j, prio in enumerate(pat):
                    rows = pl.ds(pl.multiple_of(o + (k * len(pat) + j) * piece, piece), piece)
                    start(wd_hbm.at[rows, :], wd_v.at[rows, :], S_D + i, prio)
            loop(npc // len(pat), step)

        wd_plan = [[0], [1], [2], list(range(3, n_wd))] if n_mxu >= 4 else [list(range(n_wd)), [], [], []]

        start(x_hbm, x_v, S_X, 0)
        start(c_hbm, c_v, S_C, 0)
        issue_mod()
        for g in range(LOOK):
            issue_w3(wq_hbm, wq_v, S_Q, g)

        wait_filled(c_v, S_C)
        wait_filled(x_v, S_X)
        cvec = jnp.broadcast_to(c_v[...].astype(F32), (8, M))
        sc = (cvec * jax.nn.sigmoid(cvec)).astype(BF16)
        x0 = jnp.broadcast_to(x_v[0].astype(F32), (8, M))
        ln0 = _layernorm(x0)
        wait_filled(wmod_v, S_MOD)
        mod = jnp.dot(sc, wmod_v[...], preferred_element_type=F32)
        sa, ca, ga, sb, cb, gb = (mod[:, i * M:(i + 1) * M] for i in range(6))
        h0 = ln0 * (1.0 + ca) + sa
        hb_v[...] = jnp.broadcast_to(h0[0:1, :], (128, M)).T

        def q_group(g, acc):
            issue_w3(wuk_hbm, wuk_v, S_UK, g)
            wait_w3(wq_v, S_Q, g)

            def q_part(k, acc):
                for j in range(W3_S):
                    for t in range(W3_R):
                        acc = acc + (hb_v[pl.ds(w3_row(g, k, j) + t, 1), :]
                                     * w3_at(wq_v, g, k, j, t).astype(F32))
                return acc

            return lax.fori_loop(0, w3_steps, q_part, acc)

        q = lax.fori_loop(0, NG, q_group, jnp.zeros((H, D), F32)) * scale

        lane = lax.broadcasted_iota(jnp.int32, (H, 128), 1)

        def qa_group(g, accs):
            issue_kv(g)
            wait_w3(wuk_v, S_UK, g)
            lane_rel = lane - g * w3_per
            accs = list(accs)
            for k in range(w3_steps):
                for j in range(W3_S):
                    for t in range(W3_R):
                        blk, ln = divmod(w3_row(0, k, j) + t, 128)
                        col = jnp.sum(q * w3_at(wuk_v, g, k, j, t).astype(F32), axis=1,
                                      keepdims=True)
                        accs[blk] = jnp.where(lane_rel == ln, col, accs[blk])
            return tuple(accs)

        accs = lax.fori_loop(0, NG, qa_group, tuple(jnp.zeros((H, 128), F32) for _ in range(NG)))
        qa = jnp.concatenate(accs, axis=1).astype(BF16)

        def kv_group(b, carry):
            @pl.when(b + LOOK < n_kv)
            def _():
                issue_kv(b + LOOK)

            @pl.when(b + LOOK >= n_kv)
            def _():
                issue_w3(wuv_hbm, wuv_v, S_UV, b + LOOK - n_kv)

            slabs = pl.ds(b * (kv_steps * kv_ncp), kv_steps * kv_ncp)
            wait_filled(ckv_v.at[slabs], S_KV + b)
            m, l, acc = carry
            kv = ckv_v[slabs].reshape(BK, Dc)
            s = lax.dot_general(qa, kv, _NT, preferred_element_type=F32)
            mn = jnp.maximum(m, jnp.max(s, axis=1, keepdims=True))
            a = jnp.exp(m - mn)
            p = jnp.exp(s - mn)
            l = a * l + jnp.sum(p, axis=1, keepdims=True)
            acc = a * acc + jnp.dot(p.astype(BF16), kv, preferred_element_type=F32)
            return mn, l, acc

        init = (jnp.full((H, 1), -jnp.inf, F32), jnp.zeros((H, 1), F32), jnp.zeros((H, Dc), F32))
        _, l_fin, acc_fin = lax.fori_loop(0, n_kv, kv_group, init)
        ctxc = acc_fin / l_fin
        for i in range(NG):
            qa_v[i] = ctxc[:, i * 128:(i + 1) * 128]

        def ctx_group(g, acc):
            issue_wo(g)
            wait_w3(wuv_v, S_UV, g)
            shift = (128 - g * w3_per) % 128
            blks = [pltpu.roll(qa_v[i], shift, 1) for i in range(NG)]
            for k in range(w3_steps):
                for j in range(W3_S):
                    for t in range(W3_R):
                        blk, ln = divmod(w3_row(0, k, j) + t, 128)
                        acc = acc + blks[blk][:, ln:ln + 1] * w3_at(wuv_v, g, k, j, t).astype(F32)
            return acc

        ctx_v[...] = lax.fori_loop(0, NG, ctx_group, jnp.zeros((H, D), F32))
        heads = [j * (H // WO_S) + g * wo_per + hh
                 for g in range(NG) for hh in range(wo_per) for j in range(WO_S)]
        ctx_row = jnp.concatenate([ctx_v[h:h + 1, :] for h in heads], axis=1)
        ctx_row = jnp.broadcast_to(ctx_row, (8, H * D)).astype(BF16)

        attn = jnp.zeros((8, M), F32)
        for g in range(NG):
            issue_gu(g)
            wait_filled(wo_v.at[pl.ds(g * wo_per, wo_per)], S_O + g)
            wo_g = wo_v[g * wo_per:(g + 1) * wo_per].reshape(8 * D, M)
            attn = attn + jnp.dot(ctx_row[:, g * 8 * D:(g + 1) * 8 * D], wo_g,
                                  preferred_element_type=F32)
        x1 = x0 + ga * attn
        h1 = (_layernorm(x1) * (1.0 + cb) + sb).astype(BF16)

        gate = jnp.zeros((8, Df), F32)
        up = jnp.zeros((8, Df), F32)
        for g in range(NG):
            for i in wd_plan[g]:
                issue_wd(i)
            wait_filled(wgu_v.at[g], S_GU + g)
            hk = h1[:, g * 128:(g + 1) * 128]
            gate = gate + jnp.dot(hk, wgu_v[g, 0], preferred_element_type=F32)
            up = up + jnp.dot(hk, wgu_v[g, 1], preferred_element_type=F32)
        hid = (_gelu_tanh(gate) * up).astype(BF16)

        f0 = Df - wv_rows
        hm = jnp.broadcast_to(hid[0:1, f0:].astype(F32), (128, wv_rows)).T
        y = jnp.zeros((8, M), F32)
        for i in range(n_mxu):
            o, n = wd_offs[i], wd_chunks[i]
            wait_filled(wd_v.at[pl.ds(o, n), :], S_D + i)
            y = y + jnp.dot(hid[:, o:o + n], wd_v[o:o + n, :], preferred_element_type=F32)
        row = lax.broadcasted_iota(jnp.int32, (8, M), 0)
        acc = jnp.where(row == 0, y, 0.0)
        for i in range(n_mxu, n_wd):
            o, n = wd_offs[i], wd_chunks[i]
            wait_filled(wd_v.at[pl.ds(o, n), :], S_D + i)
            for r in range(o, o + n, 16):
                wt = wd_v[r:r + 16, :].astype(F32)
                for t in range(2):
                    mul = hm[r - f0 + 8 * t:r - f0 + 8 * t + 8, :]
                    acc = acc + wt[8 * t:8 * t + 8] * jnp.concatenate([mul] * (M // 128), axis=1)
        out = x1[0:1] + gb[0:1] * jnp.sum(acc, axis=0, keepdims=True)
        o_ref[0] = out.astype(o_ref.dtype)

    any_spec = pl.BlockSpec(memory_space=pl.ANY)
    return pl.pallas_call(
        kernel,
        out_shape=jax.ShapeDtypeStruct(A_x.shape, A_x.dtype),
        in_specs=[any_spec] * 11,
        out_specs=pl.BlockSpec(memory_space=pltpu.VMEM),
        scratch_shapes=[
            pltpu.VMEM(A_x.shape, A_x.dtype),
            pltpu.VMEM(c.shape, c.dtype),
            pltpu.VMEM(w_mod.shape, w_mod.dtype),
            pltpu.VMEM(w3_vshape, A_w_q.dtype),
            pltpu.VMEM(w3_vshape, A_w_uk.dtype),
            pltpu.VMEM((n_kv * kv_steps * kv_ncp, KV_J, KV_R, Dc), A_c_kv.dtype),
            pltpu.VMEM(w3_vshape, A_w_uv.dtype),
            pltpu.VMEM((NG * wo_per, WO_S, D, M), A_w_o.dtype),
            pltpu.VMEM((NG, 2, M // NG, Df), B_w_gate.dtype),
            pltpu.VMEM(B_w_down.shape, B_w_down.dtype),
            pltpu.VMEM((M, 128), F32),
            pltpu.VMEM((NG, H, 128), F32),
            pltpu.VMEM((H, D), F32),
        ],
        compiler_params=pltpu.CompilerParams(vmem_limit_bytes=100 * 1024 * 1024),
    )(A_x, A_c_kv.reshape(KV_S, Sk // KV_S, Dc),
      A_w_q.reshape(W3_S, w3_reg, H, D), A_w_uk.reshape(W3_S, w3_reg, H, D),
      A_w_uv.reshape(W3_S, w3_reg, H, D), A_w_o.reshape(WO_S, H // WO_S, D, M),
      B_w_gate, B_w_up, B_w_down, c, w_mod)
```
